```python
import jax
import jax.numpy as jnp

def _softmax(x, axis=-1):
    return jax.nn.softmax(x, axis=axis)

def _gelu(x):
    return jax.nn.gelu(x, approximate=True)

def _silu(x):
    return jax.nn.silu(x)

def _sigmoid(x):
    return jax.nn.sigmoid(x)

def _layernorm(x, axis=-1, eps=1e-05):
    m = jnp.mean(x, axis=axis, keepdims=True)
    v = jnp.var(x, axis=axis, keepdims=True)
    return (x - m) / jnp.sqrt(v + eps)

def _scatter_add(tgt, idx, src, axis=0):
    return tgt.at[idx].add(src)

def _segment_sum(src, seg, n):
    return jax.ops.segment_sum(src, seg, n)

class _Rng:

    def __init__(self, key):
        self._k = key

    def _next(self):
        self._k, sub = jax.random.split(self._k)
        return sub

    def normal(self, shape):
        return jax.random.normal(self._next(), shape, dtype=jnp.bfloat16)

    def randint(self, lo, hi, shape):
        return jax.random.randint(self._next(), shape, lo, hi, dtype=jnp.int32)

    def uniform(self, shape, lo=0.0, hi=1.0):
        return jax.random.uniform(self._next(), shape, jnp.bfloat16, lo, hi)

    def permutation(self, n):
        return jax.random.permutation(self._next(), n)
kernel_name = 'gated_mix__memory_aug_recurrent_mem_tr__ssm_conv_h3__prompt'

def setup_inputs():
    _rng = _Rng(jax.random.key(int.from_bytes(__import__("os").urandom(4), "little")))
    _w = lambda a: (lambda t: t.astype(jnp.bfloat16) if jnp.issubdtype(t.dtype, jnp.floating) else t)(jnp.asarray(a))

    def _A_setup():
        B, S, Dm = (1, 2048, 640)
        H, Dh = (32, 192)
        M, seg = (8, 32)
        seg = min(seg, S)
        S = S // seg * seg
        return {'x': _w((lambda *s: _rng.normal(s) * 0.05)(B, S, Dm)), 'mem0': _w((lambda *s: _rng.normal(s) * 0.05)(B, M, Dm)), 'Wq': _w((lambda *s: _rng.normal(s) * 0.05)(Dm, H, Dh) * Dm ** (-0.5)), 'Wk': _w((lambda *s: _rng.normal(s) * 0.05)(Dm, H, Dh) * Dm ** (-0.5)), 'Wv': _w((lambda *s: _rng.normal(s) * 0.05)(Dm, H, Dh) * Dm ** (-0.5)), 'Wo': _w((lambda *s: _rng.normal(s) * 0.05)(H, Dh, Dm) * (H * Dh) ** (-0.5)), 'seg_len': seg}
    _A_in = _A_setup()

    def _B_setup():
        B, S, D = (1, 2048, 640)
        ks = 4
        return {'q': _w((lambda *s: _rng.normal(s) * 0.05)(B, S, D)), 'k': _w((lambda *s: _rng.normal(s) * 0.05)(B, S, D)), 'v': _w((lambda *s: _rng.normal(s) * 0.05)(B, S, D)), 'shift_k': _w((lambda *s: _rng.normal(s) * 0.05)(D, ks) * 0.5), 'ssm_k': _w((lambda *s: _rng.normal(s) * 0.05)(D, S) * (1.0 / S ** 0.5)), 'ssm_D': _w((lambda *s: _rng.normal(s) * 0.05)(D))}
    _B_in = _B_setup()
    return {'A_x': _A_in['x'], 'A_mem0': _A_in['mem0'], 'A_Wq': _A_in['Wq'], 'A_Wk': _A_in['Wk'], 'A_Wv': _A_in['Wv'], 'A_Wo': _A_in['Wo'], 'A_seg_len': _A_in['seg_len'], 'B_q': _B_in['q'], 'B_k': _B_in['k'], 'B_v': _B_in['v'], 'B_shift_k': _B_in['shift_k'], 'B_ssm_k': _B_in['ssm_k'], 'B_ssm_D': _B_in['ssm_D'], 'gate_w': _w((lambda *s: _rng.normal(s) * 0.05)(640))}

def reference(A_x, A_mem0, A_Wq, A_Wk, A_Wv, A_Wo, A_seg_len, B_q, B_k, B_v, B_shift_k, B_ssm_k, B_ssm_D, gate_w):

    def _A_ref(x, mem0, Wq, Wk, Wv, Wo, seg_len):
        B, S, Dm = x.shape
        H, Dh = (Wq.shape[1], Wq.shape[2])
        M = mem0.shape[1]
        scale = Dh ** (-0.5)
        n_seg = S // seg_len
        L = M + seg_len
        idx = jnp.arange(L)
        mask = (idx[:, None] < M) | (idx[:, None] >= idx[None, :])
        mem = mem0
        outs = []
        for s in range(n_seg):
            xs = x[:, s * seg_len:(s + 1) * seg_len, :].copy()
            h = jnp.concatenate([mem, xs], axis=1)
            q = jnp.einsum('btd,dhe->bhte', h, Wq)
            k = jnp.einsum('btd,dhe->bhte', h, Wk)
            v = jnp.einsum('btd,dhe->bhte', h, Wv)
            scores = jnp.einsum('bhqe,bhke->bhqk', q, k) * scale
            scores = jnp.where(mask[None, None], scores, -1000000000.0)
            p = _softmax(scores, axis=-1)
            o = jnp.einsum('bhqk,bhke->bhqe', p, v)
            o = jnp.einsum('bhte,hed->btd', o, Wo)
            mem = o[:, :M, :].copy()
            outs.append(o[:, M:, :])
        return jnp.concatenate(outs, axis=1)

    def _B_ref(q, k, v, shift_k, ssm_k, ssm_D):
        B, S, D = q.shape
        ks = shift_k.shape[-1]
        k_pad = jnp.pad(k, ((0, 0), (ks - 1, 0), (0, 0)))
        k_shift = jnp.zeros_like(k)
        for t in range(ks):
            k_shift = k_shift + k_pad[:, t:t + S, :] * shift_k[:, ks - 1 - t][None, None, :]
        kv = k_shift * v
        L = 2 * S
        kv_pad = jnp.pad(kv, ((0, 0), (0, S), (0, 0)))
        kf_pad = jnp.pad(ssm_k, ((0, 0), (0, S)))
        kv_f = (lambda x, axes=(-2, -1): jnp.fft.rfft2(x.astype(jnp.float32), axes=axes))(kv_pad[:, None, :, :], axes=(1, 2))
        kf_f = (lambda x, axes=(-2, -1): jnp.fft.rfft2(x.astype(jnp.float32), axes=axes))(kf_pad[:, None, :], axes=(1, 2))
        kf_f = (lambda x, *d: x.transpose(*d))(kf_f, 1, 2, 0)
        y_f = kv_f * kf_f[None, :, :, :]
        y = (lambda x, s, axes=(-2, -1): jnp.fft.irfft2(x, s=s, axes=axes).astype(jnp.bfloat16))(y_f, (1, L), axes=(1, 2))[:, 0, :S, :]
        y = y + kv * ssm_D[None, None, :]
        return q * y
    x = A_x
    g = _sigmoid((x * gate_w).sum(-1, keepdims=True))
    a = _A_ref(x, A_mem0, A_Wq, A_Wk, A_Wv, A_Wo, A_seg_len)
    b = _B_ref(x, B_k, B_v, B_shift_k, B_ssm_k, B_ssm_D)
    return g * a + (1 - g) * b
```

```python
import functools

import jax
import jax.numpy as jnp
import numpy as np
from jax import lax
import jax.experimental.pallas as pl
import jax.experimental.pallas.tpu as pltpu

_LANES = 128
_CH = 128
_NF = 2 * _CH
_LOG2E = float(np.log2(np.e))
_F32 = jnp.float32
_BF16 = jnp.bfloat16
_NT = (((1,), (1,)), ((), ()))


def _dft_matrices():
    f = np.arange(_CH, dtype=np.float64)[:, None] + 0.5
    n = np.arange(_CH, dtype=np.float64)[None, :]
    theta = 2.0 * np.pi * f * n / _NF
    fwd = np.concatenate([np.cos(theta), -np.sin(theta)], axis=0)
    inv = fwd.T / _CH
    return fwd.astype(np.float32), np.ascontiguousarray(inv).astype(np.float32)


_FWD, _INV = _dft_matrices()


def _row_vector(ref, d):
    v = ref[...].astype(_F32)
    return jnp.concatenate([v[j:j + 1, :] for j in range(d // _LANES)], axis=1)


def _kernel(
    x_hbm, mem0_ref, wq_hbm, wk_hbm, wv_hbm, wo_hbm, k_hbm, v_hbm,
    shift_ref, ssm_hbm, ssmd_ref, gate_ref, fwd_ref, inv_ref,
    out_hbm,
    x_v, k_v, v_v, ssm_v, stage_v, wqkv_v, wo_v, u_v, w_v, c_v, g_v, kf_v, h_v, o_v,
    in_sems, w_sems, out_sems,
    *, seq, dm, heads, dh, nmem, seg,
):
    n_seg = seq // seg
    n_ch = seq // _CH
    n_pair = heads // 2
    pw = 2 * dh
    rows = nmem + seg
    n_lt = dm // _LANES

    k_cp = pltpu.make_async_copy(k_hbm, k_v.at[pl.ds(16, seq)], in_sems.at[0])
    v_cp = pltpu.make_async_copy(v_hbm, v_v, in_sems.at[1])
    s_cp = pltpu.make_async_copy(ssm_hbm, ssm_v, in_sems.at[2])
    x_cp = pltpu.make_async_copy(x_hbm, x_v, in_sems.at[3])
    w_cps = [
        pltpu.make_async_copy(w, stage_v.at[i], w_sems.at[i])
        for i, w in enumerate((wq_hbm, wk_hbm, wv_hbm, wo_hbm))
    ]
    for cp in (k_cp, v_cp, s_cp, x_cp, *w_cps):
        cp.start()

    k_v[0:16, :] = jnp.zeros((16, dm), _BF16)
    shift = shift_ref[...].astype(_F32)
    ks = shift.shape[0]
    ssm_d = _row_vector(ssmd_ref, dm)
    gate_w = _row_vector(gate_ref, dm)
    fwd = fwd_ref[...]
    inv = inv_ref[...]
    sign = (1 - 2 * (lax.broadcasted_iota(jnp.int32, (_CH, dm), 0) & 1)).astype(_F32)

    k_cp.wait()
    v_cp.wait()

    def fwd_chunk(c, carry):
        r0 = pl.multiple_of(c * _CH, _CH)
        kf_v[...] = k_v[pl.ds(r0, _CH + 16), :].astype(_F32)
        acc = kf_v[16:16 + _CH, :] * shift[0:1, :]
        for j in range(1, ks):
            acc = acc + kf_v[16 - j:16 - j + _CH, :] * shift[j:j + 1, :]
        kv = (acc * v_v[pl.ds(r0, _CH), :].astype(_F32)).astype(_BF16)
        v_v[pl.ds(r0, _CH), :] = kv
        u_v[c] = jnp.dot(fwd, kv, preferred_element_type=_F32)
        return carry

    lax.fori_loop(0, n_ch, fwd_chunk, 0)

    s_cp.wait()
    prev = None
    for j in range(n_ch):
        cur = lax.dot_general(
            fwd, ssm_v[:, j * _CH:(j + 1) * _CH], _NT, preferred_element_type=_F32)
        if prev is None:
            w_v[j] = cur
        else:
            w_v[j, 0:_CH, :] = cur[0:_CH] - sign * prev[_CH:_NF]
            w_v[j, _CH:_NF, :] = cur[_CH:_NF] + sign * prev[0:_CH]
        prev = cur

    def freq_block(i, carry):
        re = pl.multiple_of(i * 8, 8)
        im = pl.multiple_of(i * 8 + _CH, 8)
        for t in range(n_lt):
            ln = slice(t * _LANES, (t + 1) * _LANES)
            ur = [u_v[c, pl.ds(re, 8), ln] for c in range(n_ch)]
            ui = [u_v[c, pl.ds(im, 8), ln] for c in range(n_ch)]
            for a in range(n_ch - 1, -1, -1):
                yr = yi = None
                for c in range(a + 1):
                    wr = w_v[a - c, pl.ds(re, 8), ln]
                    wi = w_v[a - c, pl.ds(im, 8), ln]
                    pr = ur[c] * wr - ui[c] * wi
                    pi = ur[c] * wi + ui[c] * wr
                    yr = pr if yr is None else yr + pr
                    yi = pi if yi is None else yi + pi
                u_v[a, pl.ds(re, 8), ln] = yr
                u_v[a, pl.ds(im, 8), ln] = yi
        return carry

    lax.fori_loop(0, _CH // 8, freq_block, 0)

    x_cp.wait()

    def inv_chunk(c, carry):
        r0 = pl.multiple_of(c * _CH, _CH)
        y = jnp.dot(inv, u_v[c].astype(_BF16), preferred_element_type=_F32)
        y = y + v_v[pl.ds(r0, _CH), :].astype(_F32) * ssm_d
        xs = x_v[pl.ds(r0, _CH), :].astype(_F32)
        g = jax.nn.sigmoid(jnp.sum(xs * gate_w, axis=1, keepdims=True))
        g_v[pl.ds(r0, _CH), :] = jnp.broadcast_to(g, (_CH, _LANES))
        c_v[pl.ds(r0, _CH), :] = (1.0 - g) * (xs * y)
        return carry

    lax.fori_loop(0, n_ch, inv_chunk, 0)

    for i in range(3):
        w_cps[i].wait()

        def transpose_pair(p, carry, i=i):
            r0 = pl.multiple_of(p * pw, pw)
            wt = stage_v[i, pl.ds(r0, pw), :].T
            wqkv_v[p, :, i * pw:(i + 1) * pw] = pltpu.bitcast(wt, jnp.uint32)
            return carry

        lax.fori_loop(0, n_pair, transpose_pair, 0)

    w_cps[3].wait()

    def copy_pair(p, carry):
        r0 = pl.multiple_of(p * pw, pw)
        wo_v[p] = pltpu.bitcast(stage_v[3, pl.ds(r0, pw), :], jnp.uint32)
        return carry

    lax.fori_loop(0, n_pair, copy_pair, 0)

    h_v[0:nmem, :] = mem0_ref[...].astype(_F32)
    qi = lax.broadcasted_iota(jnp.int32, (rows, 2 * rows), 0)
    lane = lax.broadcasted_iota(jnp.int32, (rows, 2 * rows), 1)
    first = lane < rows
    kj = jnp.where(first, lane, lane - rows)
    allowed = (qi < nmem) | (qi >= kj)
    low = lax.broadcasted_iota(jnp.int32, (rows, _LANES), 1) < (dh - _LANES)
    score_scale = float(dh) ** -0.5 * _LOG2E
    masked = -1000000000.0 * _LOG2E
    zero = jnp.zeros((rows, _LANES), _F32)

    def block_diag(t):
        t0, t1, t2 = t[:, 0:128], t[:, 128:256], t[:, 256:384]
        top = jnp.concatenate([t0, jnp.where(low, t1, 0.0), zero], axis=1)
        bot = jnp.concatenate([zero, jnp.where(low, 0.0, t1), t2], axis=1)
        return jnp.concatenate([top, bot], axis=0).astype(_BF16)

    def project(h, p, i):
        w = pltpu.bitcast(wqkv_v[p, :, i * pw:(i + 1) * pw], _BF16)
        return jnp.dot(h, w, preferred_element_type=_F32)

    def probs(q, kbd):
        s = lax.dot_general(q, kbd, _NT, preferred_element_type=_F32)
        s = jnp.where(allowed, s * score_scale, masked)
        m0 = jnp.max(jnp.where(first, s, -jnp.inf), axis=1, keepdims=True)
        m1 = jnp.max(jnp.where(first, -jnp.inf, s), axis=1, keepdims=True)
        e = jnp.exp2(s - jnp.where(first, m0, m1))
        l0 = jnp.sum(jnp.where(first, e, 0.0), axis=1, keepdims=True)
        l1 = jnp.sum(jnp.where(first, 0.0, e), axis=1, keepdims=True)
        return e / jnp.where(first, l0, l1)

    def out_copy(s, slot):
        r0 = pl.multiple_of(s * seg, seg)
        return pltpu.make_async_copy(
            o_v.at[slot], out_hbm.at[pl.ds(r0, seg)], out_sems.at[slot])

    def step(s, carry):
        r0 = pl.multiple_of(s * seg, seg)
        h_v[nmem:rows, :] = x_v[pl.ds(r0, seg), :].astype(_F32)
        h = h_v[...]
        q, kbd, vbd, prob, o = {}, {}, {}, {}, {}
        acc = None

        def out_proj(acc, p):
            d = jnp.dot(o.pop(p), pltpu.bitcast(wo_v[p], _BF16), preferred_element_type=_F32)
            return d if acc is None else acc + d

        def attend(p):
            o[p] = jnp.dot(prob.pop(p), vbd.pop(p), preferred_element_type=_F32)

        for p in range(n_pair):
            kbd[p] = block_diag(project(h, p, 1))
            if p >= 1:
                prob[p - 1] = probs(q.pop(p - 1), kbd.pop(p - 1))
            q[p] = project(h, p, 0)
            if p >= 2:
                attend(p - 2)
            vbd[p] = block_diag(project(h, p, 2))
        last = n_pair - 1
        acc = out_proj(acc, 0)
        prob[last] = probs(q.pop(last), kbd.pop(last))
        acc = out_proj(acc, 1)
        attend(last - 1)
        for p in range(2, 6):
            acc = out_proj(acc, p)
        attend(last)
        for p in range(6, n_pair):
            acc = out_proj(acc, p)

        h_v[0:nmem, :] = acc[0:nmem]
        slot = s % 2

        @pl.when(s >= 2)
        def _():
            out_copy(s - 2, slot).wait()

        g = g_v[pl.ds(r0, seg), :]
        g = jnp.concatenate([g] * n_lt, axis=1)
        o_v[slot] = (g * acc[nmem:rows] + c_v[pl.ds(r0, seg), :]).astype(_BF16)
        out_copy(s, slot).start()
        return carry

    lax.fori_loop(0, n_seg, step, 0)
    out_copy(n_seg - 2, 0).wait()
    out_copy(n_seg - 1, 1).wait()


@functools.partial(jax.jit, static_argnames=("A_seg_len",))
def pallas_gated_mix__memory_aug_recurrent_mem_tr__ssm_conv_h3__prompt_kernel(
    A_x: jax.Array,
    A_mem0: jax.Array,
    A_Wq: jax.Array,
    A_Wk: jax.Array,
    A_Wv: jax.Array,
    A_Wo: jax.Array,
    A_seg_len: int,
    B_q: jax.Array,
    B_k: jax.Array,
    B_v: jax.Array,
    B_shift_k: jax.Array,
    B_ssm_k: jax.Array,
    B_ssm_D: jax.Array,
    gate_w: jax.Array,
):
    del B_q
    batch, seq, dm = A_x.shape
    _, heads, dh = A_Wq.shape
    nmem = A_mem0.shape[1]
    seg = int(A_seg_len)
    assert batch == 1 and dh == 192 and heads % 2 == 0 and heads >= 14
    assert seq % _CH == 0 and seq % (2 * seg) == 0 and dm % _LANES == 0
    assert nmem % 8 == 0 and seg % 16 == 0 and 2 * (nmem + seg) <= _LANES
    hd = heads * dh
    n_pair, pw, n_ch = heads // 2, 2 * dh, seq // _CH

    def head_major(w):
        return jnp.transpose(w, (1, 2, 0)).reshape(hd, dm)

    hbm = pl.BlockSpec(memory_space=pl.ANY)
    vmem = pl.BlockSpec(memory_space=pltpu.VMEM)
    out = pl.pallas_call(
        functools.partial(
            _kernel, seq=seq, dm=dm, heads=heads, dh=dh, nmem=nmem, seg=seg),
        out_shape=jax.ShapeDtypeStruct((seq, dm), A_x.dtype),
        in_specs=[hbm, vmem, hbm, hbm, hbm, hbm, hbm, hbm,
                  vmem, hbm, vmem, vmem, vmem, vmem],
        out_specs=hbm,
        scratch_shapes=[
            pltpu.VMEM((seq, dm), _BF16),
            pltpu.VMEM((seq + 16, dm), _BF16),
            pltpu.VMEM((seq, dm), _BF16),
            pltpu.VMEM((dm, seq), _BF16),
            pltpu.VMEM((4, hd, dm), _BF16),
            pltpu.VMEM((n_pair, dm // 2, 3 * pw), jnp.uint32),
            pltpu.VMEM((n_pair, pw // 2, dm), jnp.uint32),
            pltpu.VMEM((n_ch, _NF, dm), _F32),
            pltpu.VMEM((n_ch, _NF, dm), _F32),
            pltpu.VMEM((seq, dm), _F32),
            pltpu.VMEM((seq, _LANES), _F32),
            pltpu.VMEM((_CH + 16, dm), _F32),
            pltpu.VMEM((nmem + seg, dm), _F32),
            pltpu.VMEM((2, seg, dm), _BF16),
            pltpu.SemaphoreType.DMA((4,)),
            pltpu.SemaphoreType.DMA((4,)),
            pltpu.SemaphoreType.DMA((2,)),
        ],
        compiler_params=pltpu.CompilerParams(vmem_limit_bytes=120 * 1024 * 1024),
    )(
        A_x.reshape(seq, dm),
        A_mem0.reshape(nmem, dm),
        head_major(A_Wq),
        head_major(A_Wk),
        head_major(A_Wv),
        A_Wo.reshape(hd, dm),
        B_k.reshape(seq, dm),
        B_v.reshape(seq, dm),
        B_shift_k.T,
        B_ssm_k,
        B_ssm_D.reshape(dm // _LANES, _LANES),
        gate_w.reshape(dm // _LANES, _LANES),
        jnp.asarray(_FWD, _BF16),
        jnp.asarray(_INV, _BF16),
    )
    return out.reshape(batch, seq, dm)
```

```python
import functools

import jax
import jax.numpy as jnp
import numpy as np
from jax import lax
import jax.experimental.pallas as pl
import jax.experimental.pallas.tpu as pltpu

_LANES = 128
_CH = 128
_NF = 2 * _CH
_FB = 16
_PRE = 8
_MCH = 128
_HALO = 16
_PARTS = 4
_LOG2E = float(np.log2(np.e))
_F32 = jnp.float32
_BF16 = jnp.bfloat16
_U32 = jnp.uint32
_NT = (((1,), (1,)), ((), ()))


def _dft_matrices():
    f = np.arange(_CH, dtype=np.float64)[:, None] + 0.5
    n = np.arange(_CH, dtype=np.float64)[None, :]
    theta = 2.0 * np.pi * f * n / _NF
    fwd = np.concatenate([np.cos(theta), -np.sin(theta)], axis=0)
    inv = fwd.T / _CH
    return fwd.astype(np.float32), np.ascontiguousarray(inv).astype(np.float32)


_FWD, _INV = _dft_matrices()


def _row_vector(ref, d):
    v = ref[...].astype(_F32)
    return jnp.concatenate([v[j:j + 1, :] for j in range(d // _LANES)], axis=1)


def _rows(start, size, align):
    if isinstance(start, int):
        return pl.ds(start, size)
    return pl.ds(pl.multiple_of(start, align), size)


def _kernel(
    x_hbm, xseg_hbm, mem0_ref, wq_hbm, wk_hbm, wv_hbm, wo_hbm, k_hbm, v_hbm,
    shift_ref, ssm_hbm, ssmd_ref, gate_ref, fwd_ref, inv_ref,
    out_hbm,
    x_v, xp_v, k_v, v_v, ssm_v, stage_v, wo_v, wqkv_v, pre_v, act_v,
    kf_v, kprev_v, u_v, w_v, h_v, o_v,
    in_sems, b_sems, w_sems, out_sems,
    *, seq, dm, heads, dh, nmem, seg,
):
    n_seg = seq // seg
    n_ch = seq // _CH
    n_pair = heads // 2
    pw = 2 * dh
    rows = nmem + seg
    live = rows - _PRE
    n_pre = n_seg * _PRE
    n_lt = dm // _LANES
    n_slot = stage_v.shape[0]
    part = seq // _PARTS

    kv_base = n_pre // 2
    y_base = kv_base + seq // 2

    def act_load(base, row, size):
        return pltpu.bitcast(act_v[_rows(base + row // 2, size // 2, 8), :], _BF16)

    def act_store(base, row, lanes, value):
        act_v[_rows(base + row // 2, value.shape[0] // 2, 8), lanes] = pltpu.bitcast(
            value.astype(_BF16), _U32)

    xp_cp = pltpu.make_async_copy(
        xseg_hbm.at[:, pl.ds(seg - _PRE, _PRE), :], xp_v, in_sems.at[0])
    x_cp = pltpu.make_async_copy(x_hbm, x_v, in_sems.at[1])
    wo_cp = pltpu.make_async_copy(wo_hbm, wo_v, in_sems.at[2])

    def w_copies(p):
        slot = p % n_slot
        return [
            pltpu.make_async_copy(
                w.at[_rows(p * pw, pw, pw)], stage_v.at[slot, i], w_sems.at[3 * slot + i])
            for i, w in enumerate((wq_hbm, wk_hbm, wv_hbm))
        ]

    def b_copies(j):
        span = _rows(j * part, part, part)
        return [
            pltpu.make_async_copy(
                k_hbm.at[span], k_v.at[_rows(j * part + _HALO, part, _HALO)], b_sems.at[3 * j]),
            pltpu.make_async_copy(v_hbm.at[span], v_v.at[span], b_sems.at[3 * j + 1]),
            pltpu.make_async_copy(
                ssm_hbm.at[:, span], ssm_v.at[:, span], b_sems.at[3 * j + 2]),
        ]

    queue = [[xp_cp], w_copies(0), w_copies(1), w_copies(2)]
    for p in range(3, n_slot):
        queue += [b_copies(p - 3), w_copies(p)]
    queue += [b_copies(j) for j in range(n_slot - 3, _PARTS)]

    def issue(i, carry):
        for j, group in enumerate(queue):
            @pl.when(i == j)
            def _(group=group):
                for cp in group:
                    cp.start()

        return carry

    lax.fori_loop(0, len(queue), issue, 0)

    k_v[0:_HALO, :] = jnp.zeros((_HALO, dm), _BF16)
    kprev_v[...] = jnp.zeros(kprev_v.shape, _F32)

    def forward(c, slot):
        r0 = c * _CH

        def short_conv(t):
            ln = slice(t * _LANES, (t + 1) * _LANES)
            shift = shift_ref[:, ln].astype(_F32)
            kf_v[slot, t] = k_v[_rows(r0, _CH + _HALO, _CH), ln].astype(_F32)
            acc = kf_v[slot, t, _HALO:_HALO + _CH, :] * shift[0:1, :]
            for j in range(1, shift.shape[0]):
                acc = acc + kf_v[slot, t, _HALO - j:_HALO - j + _CH, :] * shift[j:j + 1, :]
            act_store(kv_base, r0, ln, acc * v_v[_rows(r0, _CH, _CH), ln].astype(_F32))

        def signal():
            u_v[c] = jnp.dot(
                fwd_ref[...], act_load(kv_base, r0, _CH), preferred_element_type=_F32)

        def window():
            cur = lax.dot_general(
                fwd_ref[...], ssm_v[:, _rows(r0, _CH, _CH)], _NT, preferred_element_type=_F32)
            odd = lax.broadcasted_iota(jnp.int32, (_CH, dm), 0) & 1
            sign = (1 - 2 * odd).astype(_F32)
            w_v[c, 0:_CH, :] = cur[0:_CH] - sign * kprev_v[_CH:_NF, :]
            w_v[c, _CH:_NF, :] = cur[_CH:_NF] + sign * kprev_v[0:_CH, :]
            kprev_v[...] = cur

        return [functools.partial(short_conv, t) for t in range(n_lt)] + [window, signal]

    def convolve(i, slot):
        del slot
        re0 = (i // n_lt) * _FB
        im0 = re0 + _CH
        re, im = _rows(re0, _FB, _FB), _rows(im0, _FB, _FB)
        ln = _rows((i % n_lt) * _LANES, _LANES, _LANES)

        def chunks(a):
            acc = [None, None]

            def add(j, u, w):
                term = (u[0] * w[0] - u[1] * w[1], u[0] * w[1] + u[1] * w[0])
                acc[j] = term if acc[j] is None else (acc[j][0] + term[0], acc[j][1] + term[1])

            w_prev = None
            for c in range(a + 1, -1, -1):
                u = u_v[c, re, ln], u_v[c, im, ln]
                w = w_v[a + 1 - c, re, ln], w_v[a + 1 - c, im, ln]
                add(1, u, w)
                if w_prev is not None:
                    add(0, u, w_prev)
                w_prev = w
            for j in range(2):
                act_store(y_base, (a + j) * _NF + re0, ln, acc[j][0])
                act_store(y_base, (a + j) * _NF + im0, ln, acc[j][1])

        return [functools.partial(chunks, a) for a in range(0, n_ch, 2)]

    tiles = [(i, t) for i in range(3) for t in range(pw // _LANES)]

    def transpose(p, i, t):
        w = stage_v[p % n_slot, i, t * _LANES:(t + 1) * _LANES, :]
        cols = slice(i * pw + t * _LANES, i * pw + (t + 1) * _LANES)
        wqkv_v[p, :, cols] = pltpu.bitcast(w.T, _U32)

    def pre_project(p, i, t, m):
        cols = slice(i * pw + t * _LANES, i * pw + (t + 1) * _LANES)
        w = pltpu.bitcast(wqkv_v[p, :, cols], _BF16)
        pre_v[p, m * _MCH:(m + 1) * _MCH, cols] = jnp.dot(
            act_load(0, m * _MCH, _MCH), w, preferred_element_type=_F32).astype(_BF16)

    def refill(p):
        @pl.when(p + n_slot < n_pair)
        def _():
            for cp in w_copies(p + n_slot):
                cp.start()

        @pl.when(p + n_slot == n_pair)
        def _():
            x_cp.start()
            wo_cp.start()

    def interleave(*streams):
        order = [((j + 0.5) / len(s), f) for s in streams for j, f in enumerate(s)]
        for _, f in sorted(order, key=lambda e: e[0]):
            f()

    def phase(p0, n, per_iter=0, work=None, ready=None, last=False):
        def body(i, carry):
            p = p0 + i
            ahead = []
            if ready is not None:
                for cp in ready(i):
                    cp.wait()
            if not last:
                for cp in w_copies(p + 1):
                    cp.wait()
                ahead = [functools.partial(transpose, p + 1, *it) for it in tiles]
            interleave(
                [functools.partial(pre_project, p, *it, m)
                 for it in tiles for m in range(n_pre // _MCH)],
                ahead,
                [f for j in range(per_iter) for f in work(i * per_iter + j, j)])
            if not last:
                refill(p + 1)
            return carry

        lax.fori_loop(0, n, body, 0)
        return p0 + n

    xp_cp.wait()
    act_store(0, 0, slice(None), xp_v[...].astype(_F32).reshape(n_pre, dm))
    for cp in w_copies(0):
        cp.wait()
    for it in tiles:
        transpose(0, *it)
    for cp in w_copies(n_slot):
        cp.start()

    n_units = _CH // _FB * n_lt
    n_conv = n_pair - 2 - _PARTS
    p0 = phase(0, 1)
    p0 = phase(p0, _PARTS, n_ch // _PARTS, forward, b_copies)
    p0 = phase(p0, n_conv, n_units // n_conv, convolve)
    phase(p0, 1, last=True)
    x_cp.wait()
    wo_cp.wait()

    h_v[0:nmem, :] = mem0_ref[...].astype(_F32)
    qi = lax.broadcasted_iota(jnp.int32, (rows, 2 * rows), 0)
    lane = lax.broadcasted_iota(jnp.int32, (rows, 2 * rows), 1)
    first = lane < rows
    kj = jnp.where(first, lane, lane - rows)
    allowed = (qi < nmem) | (qi >= kj)
    low = lax.broadcasted_iota(jnp.int32, (rows, _LANES), 1) < (dh - _LANES)
    score_scale = float(dh) ** -0.5 * _LOG2E
    masked = -1000000000.0 * _LOG2E
    zero = jnp.zeros((rows, _LANES), _F32)

    def block_diag(t):
        t0, t1, t2 = t[:, 0:128], t[:, 128:256], t[:, 256:384]
        top = jnp.concatenate([t0, jnp.where(low, t1, 0.0), zero], axis=1)
        bot = jnp.concatenate([zero, jnp.where(low, 0.0, t1), t2], axis=1)
        return jnp.concatenate([top, bot], axis=0).astype(_BF16)

    def probs(q, kbd):
        s = lax.dot_general(q, kbd, _NT, preferred_element_type=_F32)
        s = jnp.where(allowed, s * score_scale, masked)
        m0 = jnp.max(jnp.where(first, s, -jnp.inf), axis=1, keepdims=True)
        m1 = jnp.max(jnp.where(first, -jnp.inf, s), axis=1, keepdims=True)
        e = jnp.exp2(s - jnp.where(first, m0, m1))
        l0 = jnp.sum(jnp.where(first, e, 0.0), axis=1, keepdims=True)
        l1 = jnp.sum(jnp.where(first, 0.0, e), axis=1, keepdims=True)
        return e / jnp.where(first, l0, l1)

    def out_copy(s, slot):
        return pltpu.make_async_copy(
            o_v.at[slot], out_hbm.at[_rows(s * seg, seg, seg)], out_sems.at[slot])

    def step(s, carry):
        xs = x_v[_rows(s * seg, seg, seg), :].astype(_F32)
        h_v[nmem:rows, :] = xs
        h = h_v[0:live, :].astype(_BF16)
        q, kbd, vbd, prob, o = {}, {}, {}, {}, {}
        acc = None

        def project(p, i):
            cols = slice(i * pw, (i + 1) * pw)
            w = pltpu.bitcast(wqkv_v[p, :, cols], _BF16)
            head = jnp.dot(h, w, preferred_element_type=_F32)
            tail = pre_v[p, _rows(s * _PRE, _PRE, _PRE), cols].astype(_F32)
            return jnp.concatenate([head, tail], axis=0)

        def out_proj(acc, p):
            d = jnp.dot(o.pop(p), wo_v[p * pw:(p + 1) * pw, :], preferred_element_type=_F32)
            return d if acc is None else acc + d

        def attend(p):
            o[p] = jnp.dot(prob.pop(p), vbd.pop(p), preferred_element_type=_F32)

        def branch_b():
            per_chunk = _CH // seg
            inv = inv_ref[_rows((s % per_chunk) * seg, seg, seg), :]
            y = jnp.dot(
                inv, act_load(y_base, (s // per_chunk) * _NF, _NF), preferred_element_type=_F32)
            y = y + act_load(kv_base, s * seg, seg).astype(_F32) * _row_vector(ssmd_ref, dm)
            g = jax.nn.sigmoid(
                jnp.sum(xs * _row_vector(gate_ref, dm), axis=1, keepdims=True))
            return g, (1.0 - g) * (xs * y)

        for p in range(n_pair):
            kbd[p] = block_diag(project(p, 1))
            if p >= 1:
                prob[p - 1] = probs(q.pop(p - 1), kbd.pop(p - 1))
            q[p] = project(p, 0)
            if p >= 2:
                attend(p - 2)
            vbd[p] = block_diag(project(p, 2))
        last = n_pair - 1
        acc = out_proj(acc, 0)
        prob[last] = probs(q.pop(last), kbd.pop(last))
        acc = out_proj(acc, 1)
        attend(last - 1)
        g, gated_b = branch_b()
        for p in range(2, 6):
            acc = out_proj(acc, p)
        attend(last)
        for p in range(6, n_pair):
            acc = out_proj(acc, p)

        h_v[0:nmem, :] = acc[0:nmem]
        slot = s % 2

        @pl.when(s >= 2)
        def _():
            out_copy(s - 2, slot).wait()

        o_v[slot] = (g * acc[nmem:rows] + gated_b).astype(_BF16)
        out_copy(s, slot).start()
        return carry

    lax.fori_loop(0, n_seg, step, 0)
    out_copy(n_seg - 2, 0).wait()
    out_copy(n_seg - 1, 1).wait()


@functools.partial(jax.jit, static_argnames=("A_seg_len",))
def pallas_gated_mix__memory_aug_recurrent_mem_tr__ssm_conv_h3__prompt_kernel(
    A_x: jax.Array,
    A_mem0: jax.Array,
    A_Wq: jax.Array,
    A_Wk: jax.Array,
    A_Wv: jax.Array,
    A_Wo: jax.Array,
    A_seg_len: int,
    B_q: jax.Array,
    B_k: jax.Array,
    B_v: jax.Array,
    B_shift_k: jax.Array,
    B_ssm_k: jax.Array,
    B_ssm_D: jax.Array,
    gate_w: jax.Array,
):
    del B_q
    batch, seq, dm = A_x.shape
    _, heads, dh = A_Wq.shape
    nmem = A_mem0.shape[1]
    seg = int(A_seg_len)
    assert batch == 1 and dh == 192 and heads == 32 and seq == 16 * _CH and dm == 5 * _LANES
    assert _CH % seg == 0 and seg % 16 == 0 and B_shift_k.shape[1] <= _HALO
    assert nmem % 8 == 0 and 2 * (nmem + seg) <= _LANES
    hd = heads * dh
    n_pair, pw, n_ch, n_seg = heads // 2, 2 * dh, seq // _CH, seq // seg
    n_lt = dm // _LANES
    n_slot = 6

    def head_major(w):
        return jnp.transpose(w, (1, 2, 0)).reshape(hd, dm)

    hbm = pl.BlockSpec(memory_space=pl.ANY)
    vmem = pl.BlockSpec(memory_space=pltpu.VMEM)
    out = pl.pallas_call(
        functools.partial(
            _kernel, seq=seq, dm=dm, heads=heads, dh=dh, nmem=nmem, seg=seg),
        out_shape=jax.ShapeDtypeStruct((seq, dm), A_x.dtype),
        in_specs=[hbm, hbm, vmem, hbm, hbm, hbm, hbm, hbm, hbm,
                  vmem, hbm, vmem, vmem, vmem, vmem],
        out_specs=hbm,
        scratch_shapes=[
            pltpu.VMEM((seq, dm), _BF16),
            pltpu.VMEM((n_seg, _PRE, dm), _BF16),
            pltpu.VMEM((seq + _HALO, dm), _BF16),
            pltpu.VMEM((seq, dm), _BF16),
            pltpu.VMEM((dm, seq), _BF16),
            pltpu.VMEM((n_slot, 3, pw, dm), _BF16),
            pltpu.VMEM((hd, dm), _BF16),
            pltpu.VMEM((n_pair, dm // 2, 3 * pw), _U32),
            pltpu.VMEM((n_pair, n_seg * _PRE, 3 * pw), _BF16),
            pltpu.VMEM(((n_seg * _PRE + seq + n_ch * _NF) // 2, dm), _U32),
            pltpu.VMEM((n_ch // _PARTS, n_lt, _CH + _HALO, _LANES), _F32),
            pltpu.VMEM((_NF, dm), _F32),
            pltpu.VMEM((n_ch, _NF, dm), _F32),
            pltpu.VMEM((n_ch, _NF, dm), _F32),
            pltpu.VMEM((nmem + seg, dm), _F32),
            pltpu.VMEM((2, seg, dm), _BF16),
            pltpu.SemaphoreType.DMA((3,)),
            pltpu.SemaphoreType.DMA((3 * _PARTS,)),
            pltpu.SemaphoreType.DMA((3 * n_slot,)),
            pltpu.SemaphoreType.DMA((2,)),
        ],
        compiler_params=pltpu.CompilerParams(vmem_limit_bytes=124 * 1024 * 1024),
    )(
        A_x.reshape(seq, dm),
        A_x.reshape(n_seg, seg, dm),
        A_mem0.reshape(nmem, dm),
        head_major(A_Wq),
        head_major(A_Wk),
        head_major(A_Wv),
        A_Wo.reshape(hd, dm),
        B_k.reshape(seq, dm),
        B_v.reshape(seq, dm),
        B_shift_k.T,
        B_ssm_k,
        B_ssm_D.reshape(n_lt, _LANES),
        gate_w.reshape(n_lt, _LANES),
        jnp.asarray(_FWD, _BF16),
        jnp.asarray(_INV, _BF16),
    )
    return out.reshape(batch, seq, dm)
```

```python
import functools

import jax
import jax.numpy as jnp
import numpy as np
from jax import lax
import jax.experimental.pallas as pl
import jax.experimental.pallas.tpu as pltpu

_LANES = 128
_CH = 128
_NF = 2 * _CH
_FB = 16
_PRE = 8
_MCH = 128
_HALO = 16
_PARTS = 4
_LOG2E = float(np.log2(np.e))
_F32 = jnp.float32
_BF16 = jnp.bfloat16
_U32 = jnp.uint32
_NT = (((1,), (1,)), ((), ()))


def _dft_matrices():
    f = np.arange(_CH, dtype=np.float64)[:, None] + 0.5
    n = np.arange(_CH, dtype=np.float64)[None, :]
    theta = 2.0 * np.pi * f * n / _NF
    fwd = np.concatenate([np.cos(theta), -np.sin(theta)], axis=0)
    inv = fwd.T / _CH
    return fwd.astype(np.float32), np.ascontiguousarray(inv).astype(np.float32)


_FWD, _INV = _dft_matrices()


def _row_vector(ref, d):
    v = ref[...].astype(_F32)
    return jnp.concatenate([v[j:j + 1, :] for j in range(d // _LANES)], axis=1)


def _rows(start, size, align):
    if isinstance(start, int):
        return pl.ds(start, size)
    return pl.ds(pl.multiple_of(start, align), size)


def _kernel(
    x_hbm, xseg_hbm, mem0_ref, wq_hbm, wk_hbm, wv_hbm, wo_hbm, k_hbm, v_hbm,
    shift_ref, ssm_hbm, ssmd_ref, gate_ref, fwd_ref, inv_ref,
    out_hbm,
    x_v, xp_v, k_v, v_v, ssm_v, stage_v, wo_v, wqkv_v, pre_v, act_v,
    kf_v, kprev_v, u_v, w_v, o_v,
    in_sems, b_sems, w_sems, out_sem,
    *, seq, dm, heads, dh, nmem, seg,
):
    n_seg = seq // seg
    n_ch = seq // _CH
    n_pair = heads // 2
    pw = 2 * dh
    rows = nmem + seg
    live = rows - _PRE
    n_pre = n_seg * _PRE
    n_lt = dm // _LANES
    n_slot = stage_v.shape[0]
    part = seq // _PARTS

    kv_base = n_pre // 2
    y_base = kv_base + seq // 2

    def act_load(base, row, size):
        return pltpu.bitcast(act_v[_rows(base + row // 2, size // 2, 8), :], _BF16)

    def act_store(base, row, lanes, value):
        act_v[_rows(base + row // 2, value.shape[0] // 2, 8), lanes] = pltpu.bitcast(
            value.astype(_BF16), _U32)

    xp_cp = pltpu.make_async_copy(
        xseg_hbm.at[:, pl.ds(seg - _PRE, _PRE), :], xp_v, in_sems.at[0])
    x_cp = pltpu.make_async_copy(x_hbm, x_v, in_sems.at[1])
    wo_cp = pltpu.make_async_copy(wo_hbm, wo_v, in_sems.at[2])

    def w_copies(p):
        slot = p % n_slot
        return [
            pltpu.make_async_copy(
                w.at[_rows(p * pw, pw, pw)], stage_v.at[slot, i], w_sems.at[3 * slot + i])
            for i, w in enumerate((wq_hbm, wk_hbm, wv_hbm))
        ]

    def b_copies(j):
        span = _rows(j * part, part, part)
        return [
            pltpu.make_async_copy(
                k_hbm.at[span], k_v.at[_rows(j * part + _HALO, part, _HALO)], b_sems.at[3 * j]),
            pltpu.make_async_copy(v_hbm.at[span], v_v.at[span], b_sems.at[3 * j + 1]),
            pltpu.make_async_copy(
                ssm_hbm.at[:, span], ssm_v.at[:, span], b_sems.at[3 * j + 2]),
        ]

    queue = [[xp_cp], *([cp] for cp in w_copies(0)), w_copies(1), w_copies(2)]
    for p in range(3, n_slot):
        queue += [b_copies(p - 3), w_copies(p)]
    queue += [b_copies(j) for j in range(n_slot - 3, _PARTS)]

    def issue(i, carry):
        for j, group in enumerate(queue):
            @pl.when(i == j)
            def _(group=group):
                for cp in group:
                    cp.start()

        return carry

    lax.fori_loop(0, len(queue), issue, 0)

    k_v[0:_HALO, :] = jnp.zeros((_HALO, dm), _BF16)
    kprev_v[...] = jnp.zeros(kprev_v.shape, _F32)

    def forward(c, slot):
        r0 = c * _CH

        def short_conv(t):
            ln = slice(t * _LANES, (t + 1) * _LANES)
            shift = shift_ref[:, ln].astype(_F32)
            kf_v[slot, t] = k_v[_rows(r0, _CH + _HALO, _CH), ln].astype(_F32)
            acc = kf_v[slot, t, _HALO:_HALO + _CH, :] * shift[0:1, :]
            for j in range(1, shift.shape[0]):
                acc = acc + kf_v[slot, t, _HALO - j:_HALO - j + _CH, :] * shift[j:j + 1, :]
            act_store(kv_base, r0, ln, acc * v_v[_rows(r0, _CH, _CH), ln].astype(_F32))

        def signal():
            u_v[c] = jnp.dot(
                fwd_ref[...], act_load(kv_base, r0, _CH), preferred_element_type=_F32)

        def window():
            cur = lax.dot_general(
                fwd_ref[...], ssm_v[:, _rows(r0, _CH, _CH)], _NT, preferred_element_type=_F32)
            odd = lax.broadcasted_iota(jnp.int32, (_CH, dm), 0) & 1
            sign = (1 - 2 * odd).astype(_F32)
            w_v[c, 0:_CH, :] = cur[0:_CH] - sign * kprev_v[_CH:_NF, :]
            w_v[c, _CH:_NF, :] = cur[_CH:_NF] + sign * kprev_v[0:_CH, :]
            kprev_v[...] = cur

        return [functools.partial(short_conv, t) for t in range(n_lt)] + [window, signal]

    def convolve(i, slot):
        del slot
        re0 = (i // n_lt) * _FB
        im0 = re0 + _CH
        re, im = _rows(re0, _FB, _FB), _rows(im0, _FB, _FB)
        ln = _rows((i % n_lt) * _LANES, _LANES, _LANES)

        def chunks(a):
            acc = [None, None]

            def add(j, u, w):
                term = (u[0] * w[0] - u[1] * w[1], u[0] * w[1] + u[1] * w[0])
                acc[j] = term if acc[j] is None else (acc[j][0] + term[0], acc[j][1] + term[1])

            w_prev = None
            for c in range(a + 1, -1, -1):
                u = u_v[c, re, ln], u_v[c, im, ln]
                w = w_v[a + 1 - c, re, ln], w_v[a + 1 - c, im, ln]
                add(1, u, w)
                if w_prev is not None:
                    add(0, u, w_prev)
                w_prev = w
            for j in range(2):
                act_store(y_base, (a + j) * _NF + re0, ln, acc[j][0])
                act_store(y_base, (a + j) * _NF + im0, ln, acc[j][1])

        return [functools.partial(chunks, a) for a in (0, 14, 2, 12, 4, 10, 6, 8)]

    tiles = [(i, t) for i in range(3) for t in range(pw // _LANES)]

    def transpose(p, i, t):
        w = stage_v[p % n_slot, i, t * _LANES:(t + 1) * _LANES, :]
        cols = slice(i * pw + t * _LANES, i * pw + (t + 1) * _LANES)
        wqkv_v[p, :, cols] = pltpu.bitcast(w.T, _U32)

    def pre_project(p, i, t, m, staged=False):
        cols = slice(i * pw + t * _LANES, i * pw + (t + 1) * _LANES)
        lhs = act_load(0, m * _MCH, _MCH)
        if staged:
            w = stage_v[p % n_slot, i, t * _LANES:(t + 1) * _LANES, :]
            out = lax.dot_general(lhs, w, _NT, preferred_element_type=_F32)
        else:
            w = pltpu.bitcast(wqkv_v[p, :, cols], _BF16)
            out = jnp.dot(lhs, w, preferred_element_type=_F32)
        pre_v[p, m * _MCH:(m + 1) * _MCH, cols] = out.astype(_BF16)

    def refill(p):
        @pl.when(p + n_slot < n_pair)
        def _():
            for cp in w_copies(p + n_slot):
                cp.start()

        @pl.when(p + n_slot == n_pair)
        def _():
            x_cp.start()
            wo_cp.start()

    def interleave(*streams):
        order = [((j + 0.5) / len(s), f) for s in streams for j, f in enumerate(s)]
        for _, f in sorted(order, key=lambda e: e[0]):
            f()

    def phase(p0, n, per_iter=0, work=None, ready=None):
        def body(i, carry):
            p = p0 + i
            if ready is not None:
                for cp in ready(i):
                    cp.wait()

            @pl.when(p + 1 < n_pair)
            def _():
                for cp in w_copies(p + 1):
                    cp.wait()

            interleave(
                [functools.partial(pre_project, p, *it, m)
                 for it in tiles for m in range(n_pre // _MCH)],
                [functools.partial(transpose, p + 1, *it) for it in tiles],
                [f for j in range(per_iter) for f in work(i * per_iter + j, j)])
            refill(p + 1)
            return carry

        lax.fori_loop(0, n, body, 0)
        return p0 + n

    xp_cp.wait()
    act_store(0, 0, slice(None), xp_v[...].astype(_F32).reshape(n_pre, dm))
    for i, cp in enumerate(w_copies(0)):
        cp.wait()
        mine = [it for it in tiles if it[0] == i]
        ahead = [functools.partial(transpose, 0, *it) for it in mine]
        if i == 2:
            for nxt in w_copies(1):
                nxt.wait()
            ahead += [functools.partial(transpose, 1, *it) for it in tiles]
        interleave(
            [functools.partial(pre_project, 0, *it, m, staged=True)
             for it in mine for m in range(n_pre // _MCH)],
            ahead)
    for p in range(2):
        refill(p)

    p0 = phase(1, 1)
    p0 = phase(p0, _PARTS, n_ch // _PARTS, forward, b_copies)
    n_units = _CH // _FB * n_lt
    assert n_units % (n_pair - p0) == 0
    phase(p0, n_pair - p0, n_units // (n_pair - p0), convolve)
    x_cp.wait()
    wo_cp.wait()

    qi = lax.broadcasted_iota(jnp.int32, (rows, 2 * rows), 0)
    lane = lax.broadcasted_iota(jnp.int32, (rows, 2 * rows), 1)
    first = lane < rows
    kj = jnp.where(first, lane, lane - rows)
    allowed = (qi < nmem) | (qi >= kj)
    low = lax.broadcasted_iota(jnp.int32, (rows, _LANES), 1) < (dh - _LANES)
    score_scale = float(dh) ** -0.5 * _LOG2E
    masked = -1000000000.0 * _LOG2E
    zero = jnp.zeros((rows, _LANES), _F32)

    def block_diag(t):
        t0, t1, t2 = t[:, 0:128], t[:, 128:256], t[:, 256:384]
        top = jnp.concatenate([t0, jnp.where(low, t1, 0.0), zero], axis=1)
        bot = jnp.concatenate([zero, jnp.where(low, 0.0, t1), t2], axis=1)
        return jnp.concatenate([top, bot], axis=0).astype(_BF16)

    def probs(q, kbd):
        s = lax.dot_general(q, kbd, _NT, preferred_element_type=_F32)
        s = jnp.where(allowed, s * score_scale, masked)
        m0 = jnp.max(jnp.where(first, s, -jnp.inf), axis=1, keepdims=True)
        m1 = jnp.max(jnp.where(first, -jnp.inf, s), axis=1, keepdims=True)
        e = jnp.exp2(s - jnp.where(first, m0, m1))
        l0 = jnp.sum(jnp.where(first, e, 0.0), axis=1, keepdims=True)
        l1 = jnp.sum(jnp.where(first, 0.0, e), axis=1, keepdims=True)
        return e / jnp.where(first, l0, l1)

    def step(s, mem):
        tokens = _rows(s * seg, seg, seg)
        xs = x_v[tokens, :].astype(_F32)
        h = jnp.concatenate([mem, xs[0:live - nmem]], axis=0).astype(_BF16)
        q, kbd, vbd, prob, o = {}, {}, {}, {}, {}
        acc = None

        def project(p, i):
            cols = slice(i * pw, (i + 1) * pw)
            w = pltpu.bitcast(wqkv_v[p, :, cols], _BF16)
            head = jnp.dot(h, w, preferred_element_type=_F32)
            tail = pre_v[p, _rows(s * _PRE, _PRE, _PRE), cols].astype(_F32)
            return jnp.concatenate([head, tail], axis=0)

        def out_proj(acc, p):
            d = jnp.dot(o.pop(p), wo_v[p * pw:(p + 1) * pw, :], preferred_element_type=_F32)
            return d if acc is None else acc + d

        def attend(p):
            o[p] = jnp.dot(prob.pop(p), vbd.pop(p), preferred_element_type=_F32)

        def branch_b():
            per_chunk = _CH // seg
            inv = inv_ref[_rows((s % per_chunk) * seg, seg, seg), :]
            y = jnp.dot(
                inv, act_load(y_base, (s // per_chunk) * _NF, _NF), preferred_element_type=_F32)
            y = y + act_load(kv_base, s * seg, seg).astype(_F32) * _row_vector(ssmd_ref, dm)
            g = jax.nn.sigmoid(
                jnp.sum(xs * _row_vector(gate_ref, dm), axis=1, keepdims=True))
            return g, (1.0 - g) * (xs * y)

        for p in range(n_pair):
            for op in 'KQVPS':
                if op == "K":
                    kbd[p] = block_diag(project(p, 1))
                if op == "Q":
                    q[p] = project(p, 0)
                if op == "V":
                    vbd[p] = block_diag(project(p, 2))
                if op == "S" and p >= 0:
                    prob[p - 0] = probs(q.pop(p - 0), kbd.pop(p - 0))
                if op == "P" and p >= 2:
                    attend(p - 2)
                if op == "O" and p >= 16:
                    acc = out_proj(acc, p - 16)
        for op in 'OPOBOOOOP':
            if op == "S":
                p = min(q)
                prob[p] = probs(q.pop(p), kbd.pop(p))
            if op == "P":
                attend(min(prob))
            if op == "O":
                acc = out_proj(acc, min(o))
            if op == "B":
                g, gated_b = branch_b()
        while o:
            acc = out_proj(acc, min(o))
        assert not (q or prob)

        o_v[tokens, :] = (g * acc[nmem:rows] + gated_b).astype(_BF16)
        pltpu.make_async_copy(o_v.at[tokens], out_hbm.at[tokens], out_sem).start()
        return acc[0:nmem]

    lax.fori_loop(0, n_seg, step, mem0_ref[...].astype(_F32))
    pltpu.make_async_copy(o_v, out_hbm, out_sem).wait()


@functools.partial(jax.jit, static_argnames=("A_seg_len",))
def pallas_gated_mix__memory_aug_recurrent_mem_tr__ssm_conv_h3__prompt_kernel(
    A_x: jax.Array,
    A_mem0: jax.Array,
    A_Wq: jax.Array,
    A_Wk: jax.Array,
    A_Wv: jax.Array,
    A_Wo: jax.Array,
    A_seg_len: int,
    B_q: jax.Array,
    B_k: jax.Array,
    B_v: jax.Array,
    B_shift_k: jax.Array,
    B_ssm_k: jax.Array,
    B_ssm_D: jax.Array,
    gate_w: jax.Array,
):
    del B_q
    batch, seq, dm = A_x.shape
    _, heads, dh = A_Wq.shape
    nmem = A_mem0.shape[1]
    seg = int(A_seg_len)
    assert batch == 1 and dh == 192 and heads == 32 and seq == 16 * _CH and dm == 5 * _LANES
    assert _CH % seg == 0 and seg % 16 == 0 and B_shift_k.shape[1] <= _HALO
    assert nmem % 8 == 0 and 2 * (nmem + seg) <= _LANES
    hd = heads * dh
    n_pair, pw, n_ch, n_seg = heads // 2, 2 * dh, seq // _CH, seq // seg
    n_lt = dm // _LANES
    n_slot = 6

    def head_major(w):
        return jnp.transpose(w, (1, 2, 0)).reshape(hd, dm)

    hbm = pl.BlockSpec(memory_space=pl.ANY)
    vmem = pl.BlockSpec(memory_space=pltpu.VMEM)
    out = pl.pallas_call(
        functools.partial(
            _kernel, seq=seq, dm=dm, heads=heads, dh=dh, nmem=nmem, seg=seg),
        out_shape=jax.ShapeDtypeStruct((seq, dm), A_x.dtype),
        in_specs=[hbm, hbm, vmem, hbm, hbm, hbm, hbm, hbm, hbm,
                  vmem, hbm, vmem, vmem, vmem, vmem],
        out_specs=hbm,
        scratch_shapes=[
            pltpu.VMEM((seq, dm), _BF16),
            pltpu.VMEM((n_seg, _PRE, dm), _BF16),
            pltpu.VMEM((seq + _HALO, dm), _BF16),
            pltpu.VMEM((seq, dm), _BF16),
            pltpu.VMEM((dm, seq), _BF16),
            pltpu.VMEM((n_slot, 3, pw, dm), _BF16),
            pltpu.VMEM((hd, dm), _BF16),
            pltpu.VMEM((n_pair + 1, dm // 2, 3 * pw), _U32),
            pltpu.VMEM((n_pair, n_seg * _PRE, 3 * pw), _BF16),
            pltpu.VMEM(((n_seg * _PRE + seq + n_ch * _NF) // 2, dm), _U32),
            pltpu.VMEM((n_ch // _PARTS, n_lt, _CH + _HALO, _LANES), _F32),
            pltpu.VMEM((_NF, dm), _F32),
            pltpu.VMEM((n_ch, _NF, dm), _F32),
            pltpu.VMEM((n_ch, _NF, dm), _F32),
            pltpu.VMEM((seq, dm), _BF16),
            pltpu.SemaphoreType.DMA((3,)),
            pltpu.SemaphoreType.DMA((3 * _PARTS,)),
            pltpu.SemaphoreType.DMA((3 * n_slot,)),
            pltpu.SemaphoreType.DMA(()),
        ],
        compiler_params=pltpu.CompilerParams(vmem_limit_bytes=124 * 1024 * 1024),
    )(
        A_x.reshape(seq, dm),
        A_x.reshape(n_seg, seg, dm),
        A_mem0.reshape(nmem, dm),
        head_major(A_Wq),
        head_major(A_Wk),
        head_major(A_Wv),
        A_Wo.reshape(hd, dm),
        B_k.reshape(seq, dm),
        B_v.reshape(seq, dm),
        B_shift_k.T,
        B_ssm_k,
        B_ssm_D.reshape(n_lt, _LANES),
        gate_w.reshape(n_lt, _LANES),
        jnp.asarray(_FWD, _BF16),
        jnp.asarray(_INV, _BF16),
    )
    return out.reshape(batch, seq, dm)
```

```python
import functools

import jax
import jax.numpy as jnp
import numpy as np
from jax import lax
import jax.experimental.pallas as pl
import jax.experimental.pallas.tpu as pltpu

_LANES = 128
_CH = 128
_NF = 2 * _CH
_FB = 16
_PRE = 8
_MCH = 128
_HALO = 16
_PARTS = 4
_LOG2E = float(np.log2(np.e))
_F32 = jnp.float32
_BF16 = jnp.bfloat16
_U32 = jnp.uint32
_NT = (((1,), (1,)), ((), ()))


def _dft_matrices():
    f = np.arange(_CH, dtype=np.float64)[:, None] + 0.5
    n = np.arange(_CH, dtype=np.float64)[None, :]
    theta = 2.0 * np.pi * f * n / _NF
    fwd = np.concatenate([np.cos(theta), -np.sin(theta)], axis=0)
    inv = fwd.T / _CH
    return fwd.astype(np.float32), np.ascontiguousarray(inv).astype(np.float32)


_FWD, _INV = _dft_matrices()


def _row_vector(ref, d):
    v = ref[...].astype(_F32)
    return jnp.concatenate([v[j:j + 1, :] for j in range(d // _LANES)], axis=1)


def _rows(start, size, align):
    if isinstance(start, int):
        return pl.ds(start, size)
    return pl.ds(pl.multiple_of(start, align), size)


def _kernel(
    x_hbm, xseg_hbm, mem0_ref, wq_hbm, wk_hbm, wv_hbm, wo_hbm, k_hbm, v_hbm,
    shift_ref, ssm_hbm, ssmd_ref, gate_ref, fwd_ref, inv_ref,
    out_hbm,
    x_v, xp_v, k_v, v_v, ssm_v, stage_v, wo_v, wqkv_v, pre0_v, pre1_v, pre2_v, act_v,
    kf_v, kprev_v, u_v, w_v, o_v,
    in_sems, b_sems, w_sems, out_sem,
    *, seq, dm, heads, dh, nmem, seg,
):
    n_seg = seq // seg
    n_ch = seq // _CH
    n_pair = heads // 2
    pw = 2 * dh
    rows = nmem + seg
    live = rows - _PRE
    n_pre = n_seg * _PRE
    n_lt = dm // _LANES
    n_slot = stage_v.shape[0]
    part = seq // _PARTS

    kv_base = n_pre // 2
    pre_v = (pre0_v, pre1_v, pre2_v)
    pre_rows = n_pre // 2
    pre_base = n_lt * pre_rows
    y_base = pre_base + 3 * n_pair * pre_rows

    def act_load(base, row, size):
        return pltpu.bitcast(act_v[_rows(base + row // 2, size // 2, 8), :], _BF16)

    def act_store(base, row, lanes, value):
        act_v[_rows(base + row // 2, value.shape[0] // 2, 8), lanes] = pltpu.bitcast(
            value.astype(_BF16), _U32)

    xp_cp = pltpu.make_async_copy(
        xseg_hbm.at[:, pl.ds(seg - _PRE, _PRE), :], xp_v, in_sems.at[0])
    x_cp = pltpu.make_async_copy(x_hbm, x_v, in_sems.at[1])
    wo_cp = pltpu.make_async_copy(wo_hbm, wo_v, in_sems.at[2])

    def w_copies(p):
        slot = p % n_slot
        return [
            pltpu.make_async_copy(
                w.at[_rows(p * pw, pw, pw)], stage_v.at[slot, i], w_sems.at[3 * slot + i])
            for i, w in enumerate((wq_hbm, wk_hbm, wv_hbm))
        ]

    def b_copies(j):
        span = _rows(j * part, part, part)
        return [
            pltpu.make_async_copy(
                k_hbm.at[span], k_v.at[_rows(j * part + _HALO, part, _HALO)], b_sems.at[3 * j]),
            pltpu.make_async_copy(v_hbm.at[span], v_v.at[span], b_sems.at[3 * j + 1]),
            pltpu.make_async_copy(
                ssm_hbm.at[:, span], ssm_v.at[:, span], b_sems.at[3 * j + 2]),
        ]

    queue = [[xp_cp], *([cp] for cp in w_copies(0)), w_copies(1), w_copies(2)]
    for p in range(3, n_slot):
        queue += [b_copies(p - 3), w_copies(p)]
    queue += [b_copies(j) for j in range(n_slot - 3, _PARTS)]

    def issue(i, carry):
        for j, group in enumerate(queue):
            @pl.when(i == j)
            def _(group=group):
                for cp in group:
                    cp.start()

        return carry

    lax.fori_loop(0, len(queue), issue, 0)

    k_v[0:_HALO, :] = jnp.zeros((_HALO, dm), _BF16)
    kprev_v[...] = jnp.zeros(kprev_v.shape, _F32)

    def forward(c, slot):
        r0 = c * _CH

        def short_conv(t):
            ln = slice(t * _LANES, (t + 1) * _LANES)
            shift = shift_ref[:, ln].astype(_F32)
            kf_v[slot, t] = k_v[_rows(r0, _CH + _HALO, _CH), ln].astype(_F32)
            acc = kf_v[slot, t, _HALO:_HALO + _CH, :] * shift[0:1, :]
            for j in range(1, shift.shape[0]):
                acc = acc + kf_v[slot, t, _HALO - j:_HALO - j + _CH, :] * shift[j:j + 1, :]
            act_store(kv_base, r0, ln, acc * v_v[_rows(r0, _CH, _CH), ln].astype(_F32))

        def signal():
            u_v[c] = jnp.dot(
                fwd_ref[...], act_load(kv_base, r0, _CH), preferred_element_type=_F32)

        def window():
            cur = lax.dot_general(
                fwd_ref[...], ssm_v[:, _rows(r0, _CH, _CH)], _NT, preferred_element_type=_F32)
            odd = lax.broadcasted_iota(jnp.int32, (_CH, dm), 0) & 1
            sign = (1 - 2 * odd).astype(_F32)
            w_v[c, 0:_CH, :] = cur[0:_CH] - sign * kprev_v[_CH:_NF, :]
            w_v[c, _CH:_NF, :] = cur[_CH:_NF] + sign * kprev_v[0:_CH, :]
            kprev_v[...] = cur

        return [functools.partial(short_conv, t) for t in range(n_lt)] + [window, signal]

    def convolve(i, slot):
        del slot
        re0 = (i // n_lt) * _FB
        im0 = re0 + _CH
        re, im = _rows(re0, _FB, _FB), _rows(im0, _FB, _FB)
        ln = _rows((i % n_lt) * _LANES, _LANES, _LANES)

        def chunks(a):
            acc = [None, None]

            def add(j, u, w):
                term = (u[0] * w[0] - u[1] * w[1], u[0] * w[1] + u[1] * w[0])
                acc[j] = term if acc[j] is None else (acc[j][0] + term[0], acc[j][1] + term[1])

            w_prev = None
            for c in range(a + 1, -1, -1):
                u = u_v[c, re, ln], u_v[c, im, ln]
                w = w_v[a + 1 - c, re, ln], w_v[a + 1 - c, im, ln]
                add(1, u, w)
                if w_prev is not None:
                    add(0, u, w_prev)
                w_prev = w
            for j in range(2):
                dst = _rows(y_base + (((i % n_lt) * n_ch + a + j) * _CH + re0) // 2, _FB // 2, 8)
                for r in range(2):
                    pre_v[r][dst, :] = pltpu.bitcast(acc[j][r].astype(_BF16), _U32)

        return [functools.partial(chunks, a) for a in range(0, n_ch, 2)]

    tiles = [(i, t) for i in range(3) for t in range(pw // _LANES)]

    def transpose(p, i, t):
        w = stage_v[p % n_slot, i, t * _LANES:(t + 1) * _LANES, :]
        cols = slice(i * pw + t * _LANES, i * pw + (t + 1) * _LANES)
        wqkv_v[p, :, cols] = pltpu.bitcast(w.T, _U32)

    def pre_project(p, i, t, m, staged=False, tight=False):
        cols = slice(i * pw + t * _LANES, i * pw + (t + 1) * _LANES)
        r0, n = m * _MCH // 2, _MCH // 2
        if tight:
            lhs = pltpu.bitcast(jnp.concatenate(
                [pre_v[t][j * pre_rows + r0:j * pre_rows + r0 + n, :] for j in range(n_lt)],
                axis=1), _BF16)
        else:
            lhs = act_load(0, m * _MCH, _MCH)
        if staged:
            w = stage_v[p % n_slot, i, t * _LANES:(t + 1) * _LANES, :]
            out = lax.dot_general(lhs, w, _NT, preferred_element_type=_F32)
        else:
            w = pltpu.bitcast(wqkv_v[p, :, cols], _BF16)
            out = jnp.dot(lhs, w, preferred_element_type=_F32)
        pre_v[t][_rows(pre_base + (3 * p + i) * pre_rows + r0, n, n), :] = pltpu.bitcast(
            out.astype(_BF16), _U32)

    def refill(p):
        @pl.when(p + n_slot < n_pair)
        def _():
            for cp in w_copies(p + n_slot):
                cp.start()

        @pl.when(p + n_slot == n_pair)
        def _():
            x_cp.start()
            wo_cp.start()

    def interleave(*streams):
        order = [((j + 0.5) / len(s), f) for s in streams for j, f in enumerate(s)]
        for _, f in sorted(order, key=lambda e: e[0]):
            f()

    def phase(p0, n, per_iter=0, work=None, ready=None, tight=False):
        def body(i, carry):
            p = p0 + i
            if ready is not None:
                for cp in ready(i):
                    cp.wait()

            @pl.when(p + 1 < n_pair)
            def _():
                for cp in w_copies(p + 1):
                    cp.wait()

            interleave(
                [functools.partial(pre_project, p, *it, m, tight=tight)
                 for m in range(n_pre // _MCH) for it in tiles] if tight else
                [functools.partial(pre_project, p, *it, m)
                 for it in tiles for m in range(n_pre // _MCH)],
                [functools.partial(transpose, p + 1, *it) for it in tiles],
                [f for j in range(per_iter) for f in work(i * per_iter + j, j)])
            refill(p + 1)
            return carry

        lax.fori_loop(0, n, body, 0)
        return p0 + n

    xp_cp.wait()
    xq = pltpu.bitcast(xp_v[...].astype(_F32).reshape(n_pre, dm).astype(_BF16), _U32)
    act_v[0:pre_rows, :] = xq
    for ref in pre_v:
        for j in range(n_lt):
            ref[j * pre_rows:(j + 1) * pre_rows, :] = xq[:, j * _LANES:(j + 1) * _LANES]
    for i, cp in enumerate(w_copies(0)):
        cp.wait()
        mine = [it for it in tiles if it[0] == i]
        ahead = [functools.partial(transpose, 0, *it) for it in mine]
        if i == 2:
            for nxt in w_copies(1):
                nxt.wait()
            ahead += [functools.partial(transpose, 1, *it) for it in tiles]
        interleave(
            [functools.partial(pre_project, 0, *it, m, staged=True)
             for m in range(n_pre // _MCH) for it in mine],
            ahead)
    for p in range(2):
        refill(p)

    p0 = phase(1, 1)
    p0 = phase(p0, _PARTS, n_ch // _PARTS, forward, b_copies)
    n_units = _CH // _FB * n_lt
    assert n_units % (n_pair - p0) == 0
    phase(p0, n_pair - p0, n_units // (n_pair - p0), convolve, tight=True)
    x_cp.wait()
    wo_cp.wait()

    qi = lax.broadcasted_iota(jnp.int32, (rows, 2 * rows), 0)
    lane = lax.broadcasted_iota(jnp.int32, (rows, 2 * rows), 1)
    first = lane < rows
    kj = jnp.where(first, lane, lane - rows)
    allowed = (qi < nmem) | (qi >= kj)
    low = lax.broadcasted_iota(jnp.int32, (rows, _LANES), 1) < (dh - _LANES)
    score_scale = float(dh) ** -0.5 * _LOG2E
    masked = -1000000000.0 * _LOG2E
    zero = jnp.zeros((rows, _LANES), _F32)

    def block_diag(t):
        t0, t1, t2 = t[:, 0:128], t[:, 128:256], t[:, 256:384]
        top = jnp.concatenate([t0, jnp.where(low, t1, 0.0), zero], axis=1)
        bot = jnp.concatenate([zero, jnp.where(low, 0.0, t1), t2], axis=1)
        return jnp.concatenate([top, bot], axis=0).astype(_BF16)

    def probs(q, kbd):
        s = lax.dot_general(q, kbd, _NT, preferred_element_type=_F32)
        s = jnp.where(allowed, s * score_scale, masked)
        m0 = jnp.max(jnp.where(first, s, -jnp.inf), axis=1, keepdims=True)
        m1 = jnp.max(jnp.where(first, -jnp.inf, s), axis=1, keepdims=True)
        e = jnp.exp2(s - jnp.where(first, m0, m1))
        l0 = jnp.sum(jnp.where(first, e, 0.0), axis=1, keepdims=True)
        l1 = jnp.sum(jnp.where(first, 0.0, e), axis=1, keepdims=True)
        return e / jnp.where(first, l0, l1)

    per_chunk = _CH // seg

    def step(chunk, j, mem):
        s = chunk * per_chunk + j
        tokens = _rows(s * seg, seg, seg)
        xs = x_v[tokens, :].astype(_F32)
        h = jnp.concatenate([mem, xs[0:live - nmem]], axis=0).astype(_BF16)
        vbd, prob, o = {}, {}, {}
        acc = None

        def project(p, i):
            cols = slice(i * pw, (i + 1) * pw)
            w = pltpu.bitcast(wqkv_v[p, :, cols], _BF16)
            head = jnp.dot(h, w, preferred_element_type=_F32)
            done = _rows(pre_base + (3 * p + i) * pre_rows + s * (_PRE // 2), _PRE // 2, _PRE // 2)
            tail = jnp.concatenate([ref[done, :] for ref in pre_v], axis=1)
            tail = pltpu.bitcast(tail, _BF16).astype(_F32)
            return jnp.concatenate([head, tail], axis=0)

        def out_proj(acc, p):
            d = jnp.dot(o.pop(p), wo_v[p * pw:(p + 1) * pw, :], preferred_element_type=_F32)
            return d if acc is None else acc + d

        def attend(p):
            o[p] = jnp.dot(prob.pop(p), vbd.pop(p), preferred_element_type=_F32)

        def branch_b():
            inv = inv_ref[j * seg:(j + 1) * seg, :]
            y = jnp.dot(
                inv, pltpu.bitcast(jnp.concatenate([jnp.concatenate([
                    pre_v[r][_rows(y_base + (t * n_ch + chunk) * (_CH // 2), _CH // 2, _CH // 2), :]
                    for t in range(n_lt)], axis=1) for r in range(2)], axis=0), _BF16), preferred_element_type=_F32)
            y = y + act_load(kv_base, s * seg, seg).astype(_F32) * _row_vector(ssmd_ref, dm)
            g = jax.nn.sigmoid(
                jnp.sum(xs * _row_vector(gate_ref, dm), axis=1, keepdims=True))
            return g, (1.0 - g) * (xs * y)

        for p in range(n_pair):
            kbd = block_diag(project(p, 1))
            q = project(p, 0)
            vbd[p] = block_diag(project(p, 2))
            if p >= 2:
                attend(p - 2)
            prob[p] = probs(q, kbd)
        for p in range(n_pair):
            if p == 1:
                attend(n_pair - 2)
            if p == 6:
                attend(n_pair - 1)
            acc = out_proj(acc, p)
        g, gated_b = branch_b()

        o_v[tokens, :] = (g * acc[nmem:rows] + gated_b).astype(_BF16)
        pltpu.make_async_copy(o_v.at[tokens], out_hbm.at[tokens], out_sem).start()
        return acc[0:nmem]

    def segments(chunk, mem):
        for j in range(per_chunk):
            mem = step(chunk, j, mem)
        return mem

    lax.fori_loop(0, n_ch, segments, mem0_ref[...].astype(_F32))
    pltpu.make_async_copy(o_v, out_hbm, out_sem).wait()


@functools.partial(jax.jit, static_argnames=("A_seg_len",))
def pallas_gated_mix__memory_aug_recurrent_mem_tr__ssm_conv_h3__prompt_kernel(
    A_x: jax.Array,
    A_mem0: jax.Array,
    A_Wq: jax.Array,
    A_Wk: jax.Array,
    A_Wv: jax.Array,
    A_Wo: jax.Array,
    A_seg_len: int,
    B_q: jax.Array,
    B_k: jax.Array,
    B_v: jax.Array,
    B_shift_k: jax.Array,
    B_ssm_k: jax.Array,
    B_ssm_D: jax.Array,
    gate_w: jax.Array,
):
    del B_q
    batch, seq, dm = A_x.shape
    _, heads, dh = A_Wq.shape
    nmem = A_mem0.shape[1]
    seg = int(A_seg_len)
    assert batch == 1 and dh == 192 and heads == 32 and seq == 16 * _CH and dm == 5 * _LANES
    assert _CH % seg == 0 and seg % 16 == 0 and B_shift_k.shape[1] <= _HALO
    assert nmem % 8 == 0 and 2 * (nmem + seg) <= _LANES
    hd = heads * dh
    n_pair, pw, n_ch, n_seg = heads // 2, 2 * dh, seq // _CH, seq // seg
    n_lt = dm // _LANES
    n_slot = 6

    def head_major(w):
        return jnp.transpose(w, (1, 2, 0)).reshape(hd, dm)

    hbm = pl.BlockSpec(memory_space=pl.ANY)
    vmem = pl.BlockSpec(memory_space=pltpu.VMEM)
    out = pl.pallas_call(
        functools.partial(
            _kernel, seq=seq, dm=dm, heads=heads, dh=dh, nmem=nmem, seg=seg),
        out_shape=jax.ShapeDtypeStruct((seq, dm), A_x.dtype),
        in_specs=[hbm, hbm, vmem, hbm, hbm, hbm, hbm, hbm, hbm,
                  vmem, hbm, vmem, vmem, vmem, vmem],
        out_specs=hbm,
        scratch_shapes=[
            pltpu.VMEM((seq, dm), _BF16),
            pltpu.VMEM((n_seg, _PRE, dm), _BF16),
            pltpu.VMEM((seq + _HALO, dm), _BF16),
            pltpu.VMEM((seq, dm), _BF16),
            pltpu.VMEM((dm, seq), _BF16),
            pltpu.VMEM((n_slot, 3, pw, dm), _BF16),
            pltpu.VMEM((hd, dm), _BF16),
            pltpu.VMEM((n_pair + 1, dm // 2, 3 * pw), _U32),
            *[pltpu.VMEM(((n_lt + 3 * n_pair) * n_seg * _PRE // 2 + n_lt * seq // 2, _LANES), _U32)] * 3,
            pltpu.VMEM(((n_seg * _PRE + seq) // 2, dm), _U32),
            pltpu.VMEM((n_ch // _PARTS, n_lt, _CH + _HALO, _LANES), _F32),
            pltpu.VMEM((_NF, dm), _F32),
            pltpu.VMEM((n_ch, _NF, dm), _F32),
            pltpu.VMEM((n_ch, _NF, dm), _F32),
            pltpu.VMEM((seq, dm), _BF16),
            pltpu.SemaphoreType.DMA((3,)),
            pltpu.SemaphoreType.DMA((3 * _PARTS,)),
            pltpu.SemaphoreType.DMA((3 * n_slot,)),
            pltpu.SemaphoreType.DMA(()),
        ],
        compiler_params=pltpu.CompilerParams(vmem_limit_bytes=124 * 1024 * 1024),
    )(
        A_x.reshape(seq, dm),
        A_x.reshape(n_seg, seg, dm),
        A_mem0.reshape(nmem, dm),
        head_major(A_Wq),
        head_major(A_Wk),
        head_major(A_Wv),
        A_Wo.reshape(hd, dm),
        B_k.reshape(seq, dm),
        B_v.reshape(seq, dm),
        B_shift_k.T,
        B_ssm_k,
        B_ssm_D.reshape(n_lt, _LANES),
        gate_w.reshape(n_lt, _LANES),
        jnp.asarray(_FWD, _BF16),
        jnp.asarray(_INV, _BF16),
    )
    return out.reshape(batch, seq, dm)
```

```python
import functools

import jax
import jax.numpy as jnp
import numpy as np
from jax import lax
import jax.experimental.pallas as pl
import jax.experimental.pallas.tpu as pltpu

_LANES = 128
_CH = 128
_NF = 2 * _CH
_FB = 16
_PRE = 8
_MCH = 128
_HALO = 16
_PARTS = 4
_LOG2E = float(np.log2(np.e))
_F32 = jnp.float32
_BF16 = jnp.bfloat16
_U32 = jnp.uint32
_NT = (((1,), (1,)), ((), ()))


def _dft_matrices():
    f = np.arange(_CH, dtype=np.float64)[:, None] + 0.5
    n = np.arange(_CH, dtype=np.float64)[None, :]
    theta = 2.0 * np.pi * f * n / _NF
    fwd = np.concatenate([np.cos(theta), -np.sin(theta)], axis=0)
    inv = fwd.T / _CH
    return fwd.astype(np.float32), np.ascontiguousarray(inv).astype(np.float32)


_FWD, _INV = _dft_matrices()


def _row_vector(ref, d):
    v = ref[...].astype(_F32)
    return jnp.concatenate([v[j:j + 1, :] for j in range(d // _LANES)], axis=1)


def _rows(start, size, align):
    if isinstance(start, int):
        return pl.ds(start, size)
    return pl.ds(pl.multiple_of(start, align), size)


def _kernel(
    x_hbm, xseg_hbm, mem0_ref, wq_hbm, wk_hbm, wv_hbm, wo_hbm, k_hbm, v_hbm,
    shift_ref, ssm_hbm, ssmd_ref, gate_ref, fwd_ref, inv_ref,
    out_hbm,
    x_v, xp_v, k_v, v_v, ssm_v, stage_v, wo_v, wqkv_v, pre0_v, pre1_v, pre2_v, act_v,
    kf_v, kprev_v, u_v, w_v, o_v,
    in_sems, b_sems, w_sems, out_sem,
    *, seq, dm, heads, dh, nmem, seg,
):
    n_seg = seq // seg
    n_ch = seq // _CH
    n_pair = heads // 2
    pw = 2 * dh
    rows = nmem + seg
    live = rows - _PRE
    n_pre = n_seg * _PRE
    n_lt = dm // _LANES
    n_slot = stage_v.shape[0]
    part = seq // _PARTS

    kv_base = n_pre // 2
    pre_v = (pre0_v, pre1_v, pre2_v)
    pre_rows = n_pre // 2
    pre_base = n_lt * pre_rows
    y_base = pre_base + 3 * n_pair * pre_rows

    def act_load(base, row, size):
        return pltpu.bitcast(act_v[_rows(base + row // 2, size // 2, 8), :], _BF16)

    def act_store(base, row, lanes, value):
        act_v[_rows(base + row // 2, value.shape[0] // 2, 8), lanes] = pltpu.bitcast(
            value.astype(_BF16), _U32)

    xp_cp = pltpu.make_async_copy(
        xseg_hbm.at[:, pl.ds(seg - _PRE, _PRE), :], xp_v, in_sems.at[0])
    x_cp = pltpu.make_async_copy(x_hbm, x_v, in_sems.at[1])
    wo_cp = pltpu.make_async_copy(wo_hbm, wo_v, in_sems.at[2])

    def w_copies(p):
        slot = p % n_slot
        return [
            pltpu.make_async_copy(
                w.at[_rows(p * pw, pw, pw)], stage_v.at[slot, i], w_sems.at[3 * slot + i])
            for i, w in enumerate((wq_hbm, wk_hbm, wv_hbm))
        ]

    def b_copies(j):
        span = _rows(j * part, part, part)
        return [
            pltpu.make_async_copy(
                k_hbm.at[span], k_v.at[_rows(j * part + _HALO, part, _HALO)], b_sems.at[3 * j]),
            pltpu.make_async_copy(v_hbm.at[span], v_v.at[span], b_sems.at[3 * j + 1]),
            pltpu.make_async_copy(
                ssm_hbm.at[:, span], ssm_v.at[:, span], b_sems.at[3 * j + 2]),
        ]

    queue = [[xp_cp], *([cp] for cp in w_copies(0)), w_copies(1), w_copies(2)]
    for p in range(3, n_slot):
        queue += [b_copies(p - 3), w_copies(p)]
    queue += [b_copies(j) for j in range(n_slot - 3, _PARTS)]

    def issue(i, carry):
        for j, group in enumerate(queue):
            @pl.when(i == j)
            def _(group=group):
                for cp in group:
                    cp.start()

        return carry

    lax.fori_loop(0, len(queue), issue, 0)

    k_v[0:_HALO, :] = jnp.zeros((_HALO, dm), _BF16)
    kprev_v[...] = jnp.zeros(kprev_v.shape, _F32)

    def forward(c, slot):
        r0 = c * _CH

        def short_conv(t):
            ln = slice(t * _LANES, (t + 1) * _LANES)
            shift = shift_ref[:, ln].astype(_F32)
            k = k_v[_rows(r0, _CH + _HALO, _CH), ln].astype(_F32)
            kf_v[slot, t] = k
            acc = k[_HALO:] * shift[0:1, :]
            for j in range(1, shift.shape[0]):
                acc = acc + kf_v[slot, t, _HALO - j:_HALO - j + _CH, :] * shift[j:j + 1, :]
            act_store(kv_base, r0, ln, acc * v_v[_rows(r0, _CH, _CH), ln].astype(_F32))

        def signal():
            u_v[c] = jnp.dot(
                fwd_ref[...], act_load(kv_base, r0, _CH), preferred_element_type=_F32)

        def window():
            cur = lax.dot_general(
                fwd_ref[...], ssm_v[:, _rows(r0, _CH, _CH)], _NT, preferred_element_type=_F32)
            odd = lax.broadcasted_iota(jnp.int32, (_CH, dm), 0) & 1
            sign = (1 - 2 * odd).astype(_F32)
            w_v[c, 0:_CH, :] = cur[0:_CH] - sign * kprev_v[_CH:_NF, :]
            w_v[c, _CH:_NF, :] = cur[_CH:_NF] + sign * kprev_v[0:_CH, :]
            kprev_v[...] = cur

        return [functools.partial(short_conv, t) for t in range(n_lt)] + [window, signal]

    def convolve(i, slot):
        del slot
        re0 = (i // n_lt) * _FB
        im0 = re0 + _CH
        re, im = _rows(re0, _FB, _FB), _rows(im0, _FB, _FB)
        ln = _rows((i % n_lt) * _LANES, _LANES, _LANES)

        def chunks(group):
            acc, w = {}, {}
            for c in range(max(group), -1, -1):
                ur, ui = u_v[c, re, ln], u_v[c, im, ln]
                u = (ur + ui, ur, ui)
                for a in group:
                    if a < c:
                        continue
                    if a - c not in w:
                        wr, wi = w_v[a - c, re, ln], w_v[a - c, im, ln]
                        w[a - c] = (wr, wi - wr, wr + wi)
                    term = [x * y for x, y in zip(u, w[a - c])]
                    acc[a] = [x + y for x, y in zip(acc[a], term)] if a in acc else term
            for a, (k1, k2, k3) in acc.items():
                dst = _rows(y_base + (((i % n_lt) * n_ch + a) * _CH + re0) // 2, _FB // 2, 8)
                for ref, y in zip(pre_v, (k1 - k3, k1 + k2)):
                    ref[dst, :] = pltpu.bitcast(y.astype(_BF16), _U32)

        return [functools.partial(chunks, g) for g in [range(a, a + 4) for a in range(0, n_ch, 4)]]

    tiles = [(i, t) for i in range(3) for t in range(pw // _LANES)]

    def transpose(p, i, t):
        w = stage_v[p % n_slot, i, t * _LANES:(t + 1) * _LANES, :]
        cols = slice(i * pw + t * _LANES, i * pw + (t + 1) * _LANES)
        wqkv_v[p, :, cols] = pltpu.bitcast(w.T, _U32)

    def pre_project(p, i, t, m, staged=False, tight=False):
        cols = slice(i * pw + t * _LANES, i * pw + (t + 1) * _LANES)
        r0, n = m * _MCH // 2, _MCH // 2
        if tight:
            lhs = pltpu.bitcast(jnp.concatenate(
                [pre_v[t][j * pre_rows + r0:j * pre_rows + r0 + n, :] for j in range(n_lt)],
                axis=1), _BF16)
        else:
            lhs = act_load(0, m * _MCH, _MCH)
        if staged:
            w = stage_v[p % n_slot, i, t * _LANES:(t + 1) * _LANES, :]
            out = lax.dot_general(lhs, w, _NT, preferred_element_type=_F32)
        else:
            w = pltpu.bitcast(wqkv_v[p, :, cols], _BF16)
            out = jnp.dot(lhs, w, preferred_element_type=_F32)
        pre_v[t][_rows(pre_base + (3 * p + i) * pre_rows + r0, n, n), :] = pltpu.bitcast(
            out.astype(_BF16), _U32)

    def refill(p):
        @pl.when(p + n_slot < n_pair)
        def _():
            for cp in w_copies(p + n_slot):
                cp.start()

        @pl.when(p + n_slot == n_pair)
        def _():
            x_cp.start()
            wo_cp.start()

    def interleave(*streams):
        order = [((j + 0.5) / len(s), f) for s in streams for j, f in enumerate(s)]
        for _, f in sorted(order, key=lambda e: e[0]):
            f()

    def phase(p0, n, per_iter=0, work=None, ready=None, tight=False):
        def body(i, carry):
            p = p0 + i
            if ready is not None:
                for cp in ready(i):
                    cp.wait()

            @pl.when(p + 1 < n_pair)
            def _():
                for cp in w_copies(p + 1):
                    cp.wait()

            interleave(
                [functools.partial(pre_project, p, *it, m, tight=tight)
                 for m in range(n_pre // _MCH) for it in tiles] if tight else
                [functools.partial(pre_project, p, *it, m)
                 for it in tiles for m in range(n_pre // _MCH)],
                [functools.partial(transpose, p + 1, *it) for it in tiles],
                [f for j in range(per_iter) for f in work(i * per_iter + j, j)])
            refill(p + 1)
            return carry

        lax.fori_loop(0, n, body, 0)
        return p0 + n

    xp_cp.wait()
    xq = pltpu.bitcast(xp_v[...].astype(_F32).reshape(n_pre, dm).astype(_BF16), _U32)
    act_v[0:pre_rows, :] = xq
    for ref in pre_v:
        for j in range(n_lt):
            ref[j * pre_rows:(j + 1) * pre_rows, :] = xq[:, j * _LANES:(j + 1) * _LANES]
    for i, cp in enumerate(w_copies(0)):
        cp.wait()
        mine = [it for it in tiles if it[0] == i]
        ahead = [functools.partial(transpose, 0, *it) for it in mine]
        if i == 2:
            for nxt in w_copies(1):
                nxt.wait()
            ahead += [functools.partial(transpose, 1, *it) for it in tiles]
        interleave(
            [functools.partial(pre_project, 0, *it, m, staged=True)
             for m in range(n_pre // _MCH) for it in mine],
            ahead)
    for p in range(2):
        refill(p)

    p0 = phase(1, 1)
    p0 = phase(p0, _PARTS, n_ch // _PARTS, forward, b_copies)
    n_units = _CH // _FB * n_lt
    assert n_units % (n_pair - p0) == 0
    phase(p0, n_pair - p0, n_units // (n_pair - p0), convolve, tight=True)
    x_cp.wait()
    wo_cp.wait()

    qi = lax.broadcasted_iota(jnp.int32, (rows, 2 * rows), 0)
    lane = lax.broadcasted_iota(jnp.int32, (rows, 2 * rows), 1)
    first = lane < rows
    kj = jnp.where(first, lane, lane - rows)
    allowed = (qi < nmem) | (qi >= kj)
    low = lax.broadcasted_iota(jnp.int32, (rows, _LANES), 1) < (dh - _LANES)
    score_scale = float(dh) ** -0.5 * _LOG2E
    masked = -1000000000.0 * _LOG2E
    zero = jnp.zeros((rows, _LANES), _F32)

    def block_diag(t):
        t0, t1, t2 = t[:, 0:128], t[:, 128:256], t[:, 256:384]
        top = jnp.concatenate([t0, jnp.where(low, t1, 0.0), zero], axis=1)
        bot = jnp.concatenate([zero, jnp.where(low, 0.0, t1), t2], axis=1)
        return jnp.concatenate([top, bot], axis=0).astype(_BF16)

    def probs(q, kbd):
        s = lax.dot_general(q, kbd, _NT, preferred_element_type=_F32)
        s = jnp.where(allowed, s * score_scale, masked)
        m0 = jnp.max(jnp.where(first, s, -jnp.inf), axis=1, keepdims=True)
        m1 = jnp.max(jnp.where(first, -jnp.inf, s), axis=1, keepdims=True)
        e = jnp.exp2(s - jnp.where(first, m0, m1))
        l0 = jnp.sum(jnp.where(first, e, 0.0), axis=1, keepdims=True)
        l1 = jnp.sum(jnp.where(first, 0.0, e), axis=1, keepdims=True)
        return e / jnp.where(first, l0, l1)

    per_chunk = _CH // seg

    def step(chunk, j, mem):
        s = chunk * per_chunk + j
        tokens = _rows(s * seg, seg, seg)
        xs = x_v[tokens, :].astype(_F32)
        h = jnp.concatenate([mem, xs[0:live - nmem]], axis=0).astype(_BF16)
        vbd, prob, o = {}, {}, {}
        acc = None

        def project(p, i):
            cols = slice(i * pw, (i + 1) * pw)
            w = pltpu.bitcast(wqkv_v[p, :, cols], _BF16)
            head = jnp.dot(h, w, preferred_element_type=_F32)
            done = _rows(pre_base + (3 * p + i) * pre_rows + s * (_PRE // 2), _PRE // 2, _PRE // 2)
            tail = jnp.concatenate([ref[done, :] for ref in pre_v], axis=1)
            tail = pltpu.bitcast(tail, _BF16).astype(_F32)
            return jnp.concatenate([head, tail], axis=0)

        def out_proj(acc, p):
            d = jnp.dot(o.pop(p), wo_v[p * pw:(p + 1) * pw, :], preferred_element_type=_F32)
            return d if acc is None else acc + d

        def attend(p):
            o[p] = jnp.dot(prob.pop(p), vbd.pop(p), preferred_element_type=_F32)

        def branch_b():
            inv = inv_ref[j * seg:(j + 1) * seg, :]
            y = jnp.dot(
                inv, pltpu.bitcast(jnp.concatenate([jnp.concatenate([
                    pre_v[r][_rows(y_base + (t * n_ch + chunk) * (_CH // 2), _CH // 2, _CH // 2), :]
                    for t in range(n_lt)], axis=1) for r in range(2)], axis=0), _BF16), preferred_element_type=_F32)
            y = y + act_load(kv_base, s * seg, seg).astype(_F32) * _row_vector(ssmd_ref, dm)
            g = jax.nn.sigmoid(
                jnp.sum(xs * _row_vector(gate_ref, dm), axis=1, keepdims=True))
            return g, (1.0 - g) * (xs * y)

        for p in range(n_pair):
            kbd = block_diag(project(p, 1))
            q = project(p, 0)
            vbd[p] = block_diag(project(p, 2))
            if p >= 2:
                attend(p - 2)
            prob[p] = probs(q, kbd)
        for p in range(n_pair):
            if p == 1:
                attend(n_pair - 2)
            if p == 6:
                attend(n_pair - 1)
            acc = out_proj(acc, p)
        g, gated_b = branch_b()

        o_v[tokens, :] = (g * acc[nmem:rows] + gated_b).astype(_BF16)
        pltpu.make_async_copy(o_v.at[tokens], out_hbm.at[tokens], out_sem).start()
        return acc[0:nmem]

    def segments(chunk, mem):
        for j in range(per_chunk):
            mem = step(chunk, j, mem)
        return mem

    lax.fori_loop(0, n_ch, segments, mem0_ref[...].astype(_F32))
    pltpu.make_async_copy(o_v, out_hbm, out_sem).wait()


@functools.partial(jax.jit, static_argnames=("A_seg_len",))
def pallas_gated_mix__memory_aug_recurrent_mem_tr__ssm_conv_h3__prompt_kernel(
    A_x: jax.Array,
    A_mem0: jax.Array,
    A_Wq: jax.Array,
    A_Wk: jax.Array,
    A_Wv: jax.Array,
    A_Wo: jax.Array,
    A_seg_len: int,
    B_q: jax.Array,
    B_k: jax.Array,
    B_v: jax.Array,
    B_shift_k: jax.Array,
    B_ssm_k: jax.Array,
    B_ssm_D: jax.Array,
    gate_w: jax.Array,
):
    del B_q
    batch, seq, dm = A_x.shape
    _, heads, dh = A_Wq.shape
    nmem = A_mem0.shape[1]
    seg = int(A_seg_len)
    assert batch == 1 and dh == 192 and heads == 32 and seq == 16 * _CH and dm == 5 * _LANES
    assert _CH % seg == 0 and seg % 16 == 0 and B_shift_k.shape[1] <= _HALO
    assert nmem % 8 == 0 and 2 * (nmem + seg) <= _LANES
    hd = heads * dh
    n_pair, pw, n_ch, n_seg = heads // 2, 2 * dh, seq // _CH, seq // seg
    n_lt = dm // _LANES
    n_slot = 6

    def head_major(w):
        return jnp.transpose(w, (1, 2, 0)).reshape(hd, dm)

    hbm = pl.BlockSpec(memory_space=pl.ANY)
    vmem = pl.BlockSpec(memory_space=pltpu.VMEM)
    out = pl.pallas_call(
        functools.partial(
            _kernel, seq=seq, dm=dm, heads=heads, dh=dh, nmem=nmem, seg=seg),
        out_shape=jax.ShapeDtypeStruct((seq, dm), A_x.dtype),
        in_specs=[hbm, hbm, vmem, hbm, hbm, hbm, hbm, hbm, hbm,
                  vmem, hbm, vmem, vmem, vmem, vmem],
        out_specs=hbm,
        scratch_shapes=[
            pltpu.VMEM((seq, dm), _BF16),
            pltpu.VMEM((n_seg, _PRE, dm), _BF16),
            pltpu.VMEM((seq + _HALO, dm), _BF16),
            pltpu.VMEM((seq, dm), _BF16),
            pltpu.VMEM((dm, seq), _BF16),
            pltpu.VMEM((n_slot, 3, pw, dm), _BF16),
            pltpu.VMEM((hd, dm), _BF16),
            pltpu.VMEM((n_pair + 1, dm // 2, 3 * pw), _U32),
            *[pltpu.VMEM(((n_lt + 3 * n_pair) * n_seg * _PRE // 2 + n_lt * seq // 2, _LANES), _U32)] * 3,
            pltpu.VMEM(((n_seg * _PRE + seq) // 2, dm), _U32),
            pltpu.VMEM((n_ch // _PARTS, n_lt, _CH + _HALO, _LANES), _F32),
            pltpu.VMEM((_NF, dm), _F32),
            pltpu.VMEM((n_ch, _NF, dm), _F32),
            pltpu.VMEM((n_ch, _NF, dm), _F32),
            pltpu.VMEM((seq, dm), _BF16),
            pltpu.SemaphoreType.DMA((3,)),
            pltpu.SemaphoreType.DMA((3 * _PARTS,)),
            pltpu.SemaphoreType.DMA((3 * n_slot,)),
            pltpu.SemaphoreType.DMA(()),
        ],
        compiler_params=pltpu.CompilerParams(vmem_limit_bytes=124 * 1024 * 1024, flags={'XLA_TPU_EVENLY_DISTRIBUTE_CRITICAL_NODES': True}),
    )(
        A_x.reshape(seq, dm),
        A_x.reshape(n_seg, seg, dm),
        A_mem0.reshape(nmem, dm),
        head_major(A_Wq),
        head_major(A_Wk),
        head_major(A_Wv),
        A_Wo.reshape(hd, dm),
        B_k.reshape(seq, dm),
        B_v.reshape(seq, dm),
        B_shift_k.T,
        B_ssm_k,
        B_ssm_D.reshape(n_lt, _LANES),
        gate_w.reshape(n_lt, _LANES),
        jnp.asarray(_FWD, _BF16),
        jnp.asarray(_INV, _BF16),
    )
    return out.reshape(batch, seq, dm)
```

```python
import functools

import jax
import jax.numpy as jnp
import numpy as np
from jax import lax
import jax.experimental.pallas as pl
import jax.experimental.pallas.tpu as pltpu

_LANES = 128
_CH = 128
_NF = 2 * _CH
_FB = 16
_PRE = 8
_MCH = 128
_HALO = 16
_PARTS = 4
_LOG2E = float(np.log2(np.e))
_F32 = jnp.float32
_BF16 = jnp.bfloat16
_U32 = jnp.uint32
_NT = (((1,), (1,)), ((), ()))


def _dft_matrices():
    f = np.arange(_CH, dtype=np.float64)[:, None] + 0.5
    n = np.arange(_CH, dtype=np.float64)[None, :]
    theta = 2.0 * np.pi * f * n / _NF
    fwd = np.concatenate([np.cos(theta), -np.sin(theta)], axis=0)
    inv = fwd.T / _CH
    return fwd.astype(np.float32), np.ascontiguousarray(inv).astype(np.float32)


_FWD, _INV = _dft_matrices()


def _row_vector(ref, d):
    v = ref[...].astype(_F32)
    return jnp.concatenate([v[j:j + 1, :] for j in range(d // _LANES)], axis=1)


def _rows(start, size, align):
    if isinstance(start, int):
        return pl.ds(start, size)
    return pl.ds(pl.multiple_of(start, align), size)


def _words(value):
    return pltpu.bitcast(value.astype(_BF16), _U32)


def _kernel(
    x_hbm, xseg_hbm, mem0_ref, wq_hbm, wk_hbm, wv_hbm, wo_hbm, k_hbm, v_hbm,
    shift_ref, ssm_hbm, ssmd_ref, gate_ref, fwd_ref, inv_ref,
    out_hbm,
    x_v, xp_v, k_v, v_v, ssm_v, stage_v, wo_v, wqkv_v, pre0_v, pre1_v, pre2_v, act_v,
    kf_v, kprev_v, u_v, w_v, o_v,
    in_sems, b_sems, w_sems, out_sem,
    *, seq, dm, heads, dh, nmem, seg,
):
    n_seg = seq // seg
    n_ch = seq // _CH
    n_pair = heads // 2
    pw = 2 * dh
    rows = nmem + seg
    live = rows - _PRE
    n_pre = n_seg * _PRE
    n_lt = dm // _LANES
    n_slot = stage_v.shape[0]
    part = seq // _PARTS

    pre_v = (pre0_v, pre1_v, pre2_v)
    pre_rows = n_pre // 2
    kv_base = pre_rows
    pre_base = n_lt * pre_rows
    y_base = pre_base + 3 * n_pair * pre_rows

    def act_load(base, row, size):
        return pltpu.bitcast(act_v[_rows(base + row // 2, size // 2, 8), :], _BF16)

    xp_cp = pltpu.make_async_copy(
        xseg_hbm.at[:, pl.ds(seg - _PRE, _PRE), :], xp_v, in_sems.at[0])
    x_cp = pltpu.make_async_copy(x_hbm, x_v, in_sems.at[1])
    wo_cp = pltpu.make_async_copy(wo_hbm, wo_v, in_sems.at[2])

    def w_copies(p):
        slot = p % n_slot
        return [
            pltpu.make_async_copy(
                w.at[_rows(p * pw, pw, pw)], stage_v.at[slot, i], w_sems.at[3 * slot + i])
            for i, w in enumerate((wq_hbm, wk_hbm, wv_hbm))
        ]

    def b_copies(j):
        span = _rows(j * part, part, part)
        return [
            pltpu.make_async_copy(
                k_hbm.at[span], k_v.at[_rows(j * part + _HALO, part, _HALO)], b_sems.at[3 * j]),
            pltpu.make_async_copy(v_hbm.at[span], v_v.at[span], b_sems.at[3 * j + 1]),
            pltpu.make_async_copy(
                ssm_hbm.at[:, span], ssm_v.at[:, span], b_sems.at[3 * j + 2]),
        ]

    queue = [[xp_cp], *([cp] for cp in w_copies(0)), w_copies(1), w_copies(2)]
    for p in range(3, n_slot):
        queue += [b_copies(p - 3), w_copies(p)]
    queue += [b_copies(j) for j in range(n_slot - 3, _PARTS)]

    def issue(i, carry):
        for j, group in enumerate(queue):
            @pl.when(i == j)
            def _(group=group):
                for cp in group:
                    cp.start()

        return carry

    lax.fori_loop(0, len(queue), issue, 0)

    k_v[0:_HALO, :] = jnp.zeros((_HALO, dm), _BF16)
    kprev_v[...] = jnp.zeros(kprev_v.shape, _F32)

    def forward(c, slot):
        r0 = c * _CH

        def short_conv(t):
            ln = slice(t * _LANES, (t + 1) * _LANES)
            shift = shift_ref[:, ln].astype(_F32)
            k = k_v[_rows(r0, _CH + _HALO, _CH), ln].astype(_F32)
            kf_v[slot, t] = k
            acc = k[_HALO:] * shift[0:1, :]
            for j in range(1, shift.shape[0]):
                acc = acc + kf_v[slot, t, _HALO - j:_HALO - j + _CH, :] * shift[j:j + 1, :]
            kv = acc * v_v[_rows(r0, _CH, _CH), ln].astype(_F32)
            act_v[_rows(kv_base + r0 // 2, _CH // 2, 8), ln] = _words(kv)

        def signal():
            u_v[c] = jnp.dot(
                fwd_ref[...], act_load(kv_base, r0, _CH), preferred_element_type=_F32)

        def window():
            cur = lax.dot_general(
                fwd_ref[...], ssm_v[:, _rows(r0, _CH, _CH)], _NT, preferred_element_type=_F32)
            odd = lax.broadcasted_iota(jnp.int32, (_CH, dm), 0) & 1
            sign = (1 - 2 * odd).astype(_F32)
            w_v[c, 0:_CH, :] = cur[0:_CH] - sign * kprev_v[_CH:_NF, :]
            w_v[c, _CH:_NF, :] = cur[_CH:_NF] + sign * kprev_v[0:_CH, :]
            kprev_v[...] = cur

        return [functools.partial(short_conv, t) for t in range(n_lt)] + [window, signal]

    def convolve(i, slot):
        del slot
        re0 = (i // n_lt) * _FB
        re, im = _rows(re0, _FB, _FB), _rows(re0 + _CH, _FB, _FB)
        ln = _rows((i % n_lt) * _LANES, _LANES, _LANES)

        def chunks(group):
            acc, w = {}, {}
            for c in range(max(group), -1, -1):
                ur, ui = u_v[c, re, ln], u_v[c, im, ln]
                u = (ur + ui, ur, ui)
                for a in group:
                    if a < c:
                        continue
                    if a - c not in w:
                        wr, wi = w_v[a - c, re, ln], w_v[a - c, im, ln]
                        w[a - c] = (wr, wi - wr, wr + wi)
                    term = [x * y for x, y in zip(u, w[a - c])]
                    acc[a] = [x + y for x, y in zip(acc[a], term)] if a in acc else term
            for a, (k1, k2, k3) in acc.items():
                dst = _rows(y_base + (((i % n_lt) * n_ch + a) * _CH + re0) // 2, _FB // 2, 8)
                for ref, y in zip(pre_v, (k1 - k3, k1 + k2)):
                    ref[dst, :] = _words(y)

        return [functools.partial(chunks, range(a, a + 4)) for a in range(0, n_ch, 4)]

    tiles = [(i, t) for i in range(3) for t in range(pw // _LANES)]

    def transpose(p, i, t):
        w = stage_v[p % n_slot, i, t * _LANES:(t + 1) * _LANES, :]
        cols = slice(i * pw + t * _LANES, i * pw + (t + 1) * _LANES)
        wqkv_v[p, :, cols] = pltpu.bitcast(w.T, _U32)

    def pre_project(p, i, t, m, staged=False, tight=False):
        cols = slice(i * pw + t * _LANES, i * pw + (t + 1) * _LANES)
        r0, n = m * _MCH // 2, _MCH // 2
        if tight:
            lhs = pltpu.bitcast(jnp.concatenate(
                [pre_v[t][j * pre_rows + r0:j * pre_rows + r0 + n, :] for j in range(n_lt)],
                axis=1), _BF16)
        else:
            lhs = act_load(0, m * _MCH, _MCH)
        if staged:
            w = stage_v[p % n_slot, i, t * _LANES:(t + 1) * _LANES, :]
            out = lax.dot_general(lhs, w, _NT, preferred_element_type=_F32)
        else:
            w = pltpu.bitcast(wqkv_v[p, :, cols], _BF16)
            out = jnp.dot(lhs, w, preferred_element_type=_F32)
        pre_v[t][_rows(pre_base + (3 * p + i) * pre_rows + r0, n, n), :] = _words(out)

    def refill(p):
        @pl.when(p + n_slot < n_pair)
        def _():
            for cp in w_copies(p + n_slot):
                cp.start()

        @pl.when(p + n_slot == n_pair)
        def _():
            x_cp.start()
            wo_cp.start()

    def interleave(*streams):
        order = [((j + 0.5) / len(s), f) for s in streams for j, f in enumerate(s)]
        for _, f in sorted(order, key=lambda e: e[0]):
            f()

    def phase(p0, n, per_iter=0, work=None, ready=None, tight=False):
        def body(i, carry):
            p = p0 + i
            if ready is not None:
                for cp in ready(i):
                    cp.wait()

            @pl.when(p + 1 < n_pair)
            def _():
                for cp in w_copies(p + 1):
                    cp.wait()

            blocks = [(it, m) for it in tiles for m in range(n_pre // _MCH)]
            if tight:
                blocks.sort(key=lambda b: b[1])
            interleave(
                [functools.partial(pre_project, p, *it, m, tight=tight) for it, m in blocks],
                [functools.partial(transpose, p + 1, *it) for it in tiles],
                [f for j in range(per_iter) for f in work(i * per_iter + j, j)])
            refill(p + 1)
            return carry

        lax.fori_loop(0, n, body, 0)
        return p0 + n

    xp_cp.wait()
    xq = _words(xp_v[...].astype(_F32).reshape(n_pre, dm))
    act_v[0:pre_rows, :] = xq
    for ref in pre_v:
        for j in range(n_lt):
            ref[j * pre_rows:(j + 1) * pre_rows, :] = xq[:, j * _LANES:(j + 1) * _LANES]
    for i, cp in enumerate(w_copies(0)):
        cp.wait()
        mine = [it for it in tiles if it[0] == i]
        ahead = [functools.partial(transpose, 0, *it) for it in mine]
        if i == 2:
            for nxt in w_copies(1):
                nxt.wait()
            ahead += [functools.partial(transpose, 1, *it) for it in tiles]
        interleave(
            [functools.partial(pre_project, 0, *it, m, staged=True)
             for m in range(n_pre // _MCH) for it in mine],
            ahead)
    for p in range(2):
        refill(p)

    p0 = phase(1, 1)
    p0 = phase(p0, _PARTS, n_ch // _PARTS, forward, b_copies)
    n_units = _CH // _FB * n_lt
    assert n_units % (n_pair - p0) == 0
    phase(p0, n_pair - p0, n_units // (n_pair - p0), convolve, tight=True)
    x_cp.wait()
    wo_cp.wait()

    qi = lax.broadcasted_iota(jnp.int32, (rows, 2 * rows), 0)
    lane = lax.broadcasted_iota(jnp.int32, (rows, 2 * rows), 1)
    first = lane < rows
    kj = jnp.where(first, lane, lane - rows)
    allowed = (qi < nmem) | (qi >= kj)
    low = lax.broadcasted_iota(jnp.int32, (rows, _LANES), 1) < (dh - _LANES)
    score_scale = float(dh) ** -0.5 * _LOG2E
    masked = -1000000000.0 * _LOG2E
    zero = jnp.zeros((rows, _LANES), _F32)

    def block_diag(t):
        t0, t1, t2 = t[:, 0:128], t[:, 128:256], t[:, 256:384]
        top = jnp.concatenate([t0, jnp.where(low, t1, 0.0), zero], axis=1)
        bot = jnp.concatenate([zero, jnp.where(low, 0.0, t1), t2], axis=1)
        return jnp.concatenate([top, bot], axis=0).astype(_BF16)

    def probs(q, kbd):
        s = lax.dot_general(q, kbd, _NT, preferred_element_type=_F32)
        s = jnp.where(allowed, s * score_scale, masked)
        m0 = jnp.max(jnp.where(first, s, -jnp.inf), axis=1, keepdims=True)
        m1 = jnp.max(jnp.where(first, -jnp.inf, s), axis=1, keepdims=True)
        e = jnp.exp2(s - jnp.where(first, m0, m1))
        l0 = jnp.sum(jnp.where(first, e, 0.0), axis=1, keepdims=True)
        l1 = jnp.sum(jnp.where(first, 0.0, e), axis=1, keepdims=True)
        return e / jnp.where(first, l0, l1)

    per_chunk = _CH // seg

    def step(chunk, j, mem):
        s = chunk * per_chunk + j
        tokens = _rows(s * seg, seg, seg)
        xs = x_v[tokens, :].astype(_F32)
        h = jnp.concatenate([mem, xs[0:live - nmem]], axis=0).astype(_BF16)
        vbd, prob, o = {}, {}, {}
        acc = None

        def project(p, i):
            cols = slice(i * pw, (i + 1) * pw)
            w = pltpu.bitcast(wqkv_v[p, :, cols], _BF16)
            head = jnp.dot(h, w, preferred_element_type=_F32)
            done = _rows(pre_base + (3 * p + i) * pre_rows + s * (_PRE // 2), _PRE // 2, _PRE // 2)
            tail = jnp.concatenate([ref[done, :] for ref in pre_v], axis=1)
            tail = pltpu.bitcast(tail, _BF16).astype(_F32)
            return jnp.concatenate([head, tail], axis=0)

        def out_proj(acc, p):
            d = jnp.dot(o.pop(p), wo_v[p * pw:(p + 1) * pw, :], preferred_element_type=_F32)
            return d if acc is None else acc + d

        def attend(p):
            o[p] = jnp.dot(prob.pop(p), vbd.pop(p), preferred_element_type=_F32)

        def branch_b():
            half = _CH // 2
            spec = jnp.concatenate([
                jnp.concatenate(
                    [ref[_rows(y_base + (t * n_ch + chunk) * half, half, half), :]
                     for t in range(n_lt)], axis=1)
                for ref in pre_v[:2]], axis=0)
            y = jnp.dot(
                inv_ref[j * seg:(j + 1) * seg, :], pltpu.bitcast(spec, _BF16),
                preferred_element_type=_F32)
            y = y + act_load(kv_base, s * seg, seg).astype(_F32) * _row_vector(ssmd_ref, dm)
            g = jax.nn.sigmoid(
                jnp.sum(xs * _row_vector(gate_ref, dm), axis=1, keepdims=True))
            return g, (1.0 - g) * (xs * y)

        for p in range(n_pair):
            kbd = block_diag(project(p, 1))
            q = project(p, 0)
            vbd[p] = block_diag(project(p, 2))
            if p >= 2:
                attend(p - 2)
            prob[p] = probs(q, kbd)
        for p in range(n_pair):
            if p == 1:
                attend(n_pair - 2)
            if p == 6:
                attend(n_pair - 1)
            acc = out_proj(acc, p)
        g, gated_b = branch_b()

        o_v[tokens, :] = (g * acc[nmem:rows] + gated_b).astype(_BF16)
        pltpu.make_async_copy(o_v.at[tokens], out_hbm.at[tokens], out_sem).start()
        return acc[0:nmem]

    def segments(chunk, mem):
        for j in range(per_chunk):
            mem = step(chunk, j, mem)
        return mem

    lax.fori_loop(0, n_ch, segments, mem0_ref[...].astype(_F32))
    pltpu.make_async_copy(o_v, out_hbm, out_sem).wait()


@functools.partial(jax.jit, static_argnames=("A_seg_len",))
def pallas_gated_mix__memory_aug_recurrent_mem_tr__ssm_conv_h3__prompt_kernel(
    A_x: jax.Array,
    A_mem0: jax.Array,
    A_Wq: jax.Array,
    A_Wk: jax.Array,
    A_Wv: jax.Array,
    A_Wo: jax.Array,
    A_seg_len: int,
    B_q: jax.Array,
    B_k: jax.Array,
    B_v: jax.Array,
    B_shift_k: jax.Array,
    B_ssm_k: jax.Array,
    B_ssm_D: jax.Array,
    gate_w: jax.Array,
):
    del B_q
    batch, seq, dm = A_x.shape
    _, heads, dh = A_Wq.shape
    nmem = A_mem0.shape[1]
    seg = int(A_seg_len)
    assert batch == 1 and dh == 192 and heads == 32 and seq == 16 * _CH and dm == 5 * _LANES
    assert _CH % seg == 0 and seg % 16 == 0 and B_shift_k.shape[1] <= _HALO
    assert nmem % 8 == 0 and 2 * (nmem + seg) <= _LANES
    hd = heads * dh
    n_pair, pw, n_ch, n_seg = heads // 2, 2 * dh, seq // _CH, seq // seg
    n_lt = dm // _LANES
    n_slot = 6
    pre_words = ((n_lt + 3 * n_pair) * n_seg * _PRE + n_lt * seq) // 2

    def head_major(w):
        return jnp.transpose(w, (1, 2, 0)).reshape(hd, dm)

    hbm = pl.BlockSpec(memory_space=pl.ANY)
    vmem = pl.BlockSpec(memory_space=pltpu.VMEM)
    out = pl.pallas_call(
        functools.partial(
            _kernel, seq=seq, dm=dm, heads=heads, dh=dh, nmem=nmem, seg=seg),
        out_shape=jax.ShapeDtypeStruct((seq, dm), A_x.dtype),
        in_specs=[hbm, hbm, vmem, hbm, hbm, hbm, hbm, hbm, hbm,
                  vmem, hbm, vmem, vmem, vmem, vmem],
        out_specs=hbm,
        scratch_shapes=[
            pltpu.VMEM((seq, dm), _BF16),
            pltpu.VMEM((n_seg, _PRE, dm), _BF16),
            pltpu.VMEM((seq + _HALO, dm), _BF16),
            pltpu.VMEM((seq, dm), _BF16),
            pltpu.VMEM((dm, seq), _BF16),
            pltpu.VMEM((n_slot, 3, pw, dm), _BF16),
            pltpu.VMEM((hd, dm), _BF16),
            pltpu.VMEM((n_pair + 1, dm // 2, 3 * pw), _U32),
            *[pltpu.VMEM((pre_words, _LANES), _U32)] * 3,
            pltpu.VMEM(((n_seg * _PRE + seq) // 2, dm), _U32),
            pltpu.VMEM((n_ch // _PARTS, n_lt, _CH + _HALO, _LANES), _F32),
            pltpu.VMEM((_NF, dm), _F32),
            pltpu.VMEM((n_ch, _NF, dm), _F32),
            pltpu.VMEM((n_ch, _NF, dm), _F32),
            pltpu.VMEM((seq, dm), _BF16),
            pltpu.SemaphoreType.DMA((3,)),
            pltpu.SemaphoreType.DMA((3 * _PARTS,)),
            pltpu.SemaphoreType.DMA((3 * n_slot,)),
            pltpu.SemaphoreType.DMA(()),
        ],
        compiler_params=pltpu.CompilerParams(vmem_limit_bytes=124 * 1024 * 1024),
    )(
        A_x.reshape(seq, dm),
        A_x.reshape(n_seg, seg, dm),
        A_mem0.reshape(nmem, dm),
        head_major(A_Wq),
        head_major(A_Wk),
        head_major(A_Wv),
        A_Wo.reshape(hd, dm),
        B_k.reshape(seq, dm),
        B_v.reshape(seq, dm),
        B_shift_k.T,
        B_ssm_k,
        B_ssm_D.reshape(n_lt, _LANES),
        gate_w.reshape(n_lt, _LANES),
        jnp.asarray(_FWD, _BF16),
        jnp.asarray(_INV, _BF16),
    )
    return out.reshape(batch, seq, dm)
```
